```python
import jax
import jax.numpy as jnp

def _softmax(x, axis=-1):
    return jax.nn.softmax(x, axis=axis)
def _gelu(x):
    return jax.nn.gelu(x, approximate=True)
def _silu(x):
    return jax.nn.silu(x)
def _sigmoid(x):
    return jax.nn.sigmoid(x)
def _layernorm(x, axis=-1, eps=1e-5):
    m = jnp.mean(x, axis=axis, keepdims=True)
    v = jnp.var(x, axis=axis, keepdims=True)
    return (x - m) / jnp.sqrt(v + eps)
def _scatter_add(tgt, idx, src, axis=0):
    return tgt.at[idx].add(src)
def _segment_sum(src, seg, n):
    return jax.ops.segment_sum(src, seg, n)
class _Rng:
    def __init__(self, key):
        self._k = key
    def _next(self):
        self._k, sub = jax.random.split(self._k)
        return sub
    def normal(self, shape):
        return jax.random.normal(self._next(), shape, dtype=jnp.bfloat16)
    def randint(self, lo, hi, shape):
        return jax.random.randint(self._next(), shape, lo, hi, dtype=jnp.int32)
    def uniform(self, shape, lo=0.0, hi=1.0):
        return jax.random.uniform(self._next(), shape, jnp.bfloat16, lo, hi)
    def permutation(self, n):
        return jax.random.permutation(self._next(), n)


kernel_name = 'concat_heads__spectral_gfnet__compressed_kv_cla__prompt'

def setup_inputs():
    _rng = _Rng(jax.random.key(int.from_bytes(__import__("os").urandom(4), "little")))
    _w = (lambda a: (lambda t: t.astype(jnp.bfloat16) if jnp.issubdtype(t.dtype, jnp.floating) else t)(jnp.asarray(a)))
    def _A_setup():
        B, S, D = 1, 2048, 448
        Df = D // 2 + 1
        return {
            "x": _w((lambda *s: _rng.normal(s) * 0.05)(B, S, D)),
            "w_r": _w((lambda *s: _rng.normal(s) * 0.05)(S, Df) * 0.02),
            "w_i": _w((lambda *s: _rng.normal(s) * 0.05)(S, Df) * 0.02),
        }
    _A_in = _A_setup()

    def _B_setup():
        B, H, Sq, Sk, D, M = 1, 16, 2048, 2048, 256, 448
        Dc = 4 * D
        return {
            "x": _w((lambda *s: _rng.normal(s) * 0.05)(B, Sq, M)),
            "c_kv": _w((lambda *s: _rng.normal(s) * 0.05)(B, Sk, Dc)),
            "w_q": _w((lambda *s: _rng.normal(s) * 0.05)(M, H, D) * (M ** -0.5)),
            "w_uk": _w((lambda *s: _rng.normal(s) * 0.05)(Dc, H, D) * (Dc ** -0.5)),
            "w_uv": _w((lambda *s: _rng.normal(s) * 0.05)(Dc, H, D) * (Dc ** -0.5)),
            "w_o": _w((lambda *s: _rng.normal(s) * 0.05)(H, D, M) * ((H * D) ** -0.5)),
        }
    _B_in = _B_setup()

    return {
        "A_x": _A_in["x"],
        "A_w_r": _A_in["w_r"],
        "A_w_i": _A_in["w_i"],
        "B_x": _B_in["x"],
        "B_c_kv": _B_in["c_kv"],
        "B_w_q": _B_in["w_q"],
        "B_w_uk": _B_in["w_uk"],
        "B_w_uv": _B_in["w_uv"],
        "B_w_o": _B_in["w_o"],
    }

def reference(A_x, A_w_r, A_w_i, B_x, B_c_kv, B_w_q, B_w_uk, B_w_uv, B_w_o):
    def _A_ref(x, w_r, w_i):
        B, S, D = x.shape
        X = (lambda x, axes=(-2,-1): jnp.fft.rfft2(x.astype(jnp.float32), axes=axes))(x, axes=(-2, -1))
        W = w_r + 1j * w_i
        X = X * W
        y = (lambda x, s, axes=(-2,-1): jnp.fft.irfft2(x, s=s, axes=axes).astype(jnp.bfloat16))(X, (S, D), axes=(-2, -1))
        return y

    def _B_ref(x, c_kv, w_q, w_uk, w_uv, w_o):
        B, Sq, M = x.shape[0], x.shape[1], x.shape[2]
        Sk = c_kv.shape[1]
        H, D = w_q.shape[1], w_q.shape[2]
        q = jnp.einsum("bqm,mhd->bhqd", x, w_q)
        k = jnp.einsum("bkc,chd->bhkd", c_kv, w_uk)
        v = jnp.einsum("bkc,chd->bhkd", c_kv, w_uv)
        scores = jnp.einsum("bhqd,bhkd->bhqk", q, k) * (D ** -0.5)
        off = Sk - Sq
        qi = jnp.arange(Sq)[:, None]
        kj = jnp.arange(Sk)[None, :]
        cmask = kj <= (qi + off)
        scores = jnp.where(cmask[None, None], scores, -1e9)
        p = _softmax(scores, axis=-1)
        ctx = jnp.einsum("bhqk,bhkd->bhqd", p, v)
        return jnp.einsum("bhqd,hdm->bqm", ctx, w_o)

    a = _A_ref(A_x, A_w_r, A_w_i)
    b = _B_ref(B_x, B_c_kv, B_w_q, B_w_uk, B_w_uv, B_w_o)
    return jnp.concatenate([a, b], axis=-1)
```

```python
import functools, math
import numpy as np, jax, jax.numpy as jnp
import ml_dtypes
from jax import lax
from jax.experimental import pallas as pl
from jax.experimental.pallas import tpu as pltpu

S, M, H, D, DC = 2048, 448, 16, 256, 1024
DF = M // 2 + 1
f32, bf = jnp.float32, jnp.bfloat16
NT = (((1,), (1,)), ((), ()))
LOG2E = 1.4426950408889634
QSCALE = (D ** -0.5) * LOG2E
NEG = -1e9 * LOG2E

def _consts():
    nb = ml_dtypes.bfloat16
    d = np.arange(M, dtype=np.float64)
    f = np.arange(DF, dtype=np.float64)
    ang = 2 * np.pi * ((f[:, None] * d[None, :]) % M) / M
    cs, sn = np.cos(ang), np.sin(ang)
    FT = np.zeros((480, M))
    FT[0:128] = cs[:128]; FT[128:256] = -sn[:128]
    FT[256:256 + 97] = cs[128:]; FT[368:368 + 97] = -sn[128:]
    k1 = np.arange(16)[:, None, None]; k2 = np.arange(128)[None, :, None]; n2 = np.arange(128)[None, None, :]
    a = 2 * np.pi * ((n2 * (k1 + 16 * k2)) % S) / S
    Mr, Mi = np.cos(a), -np.sin(a)
    MF = np.concatenate([np.concatenate([Mr, -Mi], 2), np.concatenate([Mi, Mr], 2)], 1)
    MI = np.transpose(MF, (0, 2, 1)) / S
    c = np.full(DF, 2.0); c[0] = 1.0; c[-1] = 1.0
    Gc = (c[:, None] * cs) / M; Gs = -(c[:, None] * sn) / M
    G = np.zeros((512, M))
    G[0:128] = Gc[:128]; G[128:225] = Gc[128:]; G[256:384] = Gs[:128]; G[384:481] = Gs[128:]
    P = np.zeros((128, 128))
    for a_ in range(16):
        for j in range(8):
            P[a_ * 8 + j, 16 * j + a_] = 1.0
    return tuple(np.asarray(x, dtype=np.float32).astype(nb) for x in (FT, MF, MI, G, P))

_C = [math.cos(2 * math.pi * k / 16) for k in range(16)]
_S = [math.sin(2 * math.pi * k / 16) for k in range(16)]

def _cmul_tw(re, im, k, sign):
    k = k % 16
    c, s = _C[k], sign * _S[k]
    if k == 0: return re, im
    if k == 4: return (-sign * im, sign * re) if True else None
    if k == 8: return -re, -im
    if k == 12: return (sign * im, -sign * re)
    if k in (2, 6, 10, 14):
        h = math.sqrt(0.5)
        sc, ss = (1 if c > 0 else -1), (1 if s > 0 else -1)
        a = (re - im) if sc == ss else (re + im)
        b = (re + im) if sc == ss else (re - im)
        if sc == 1 and ss == 1: return (re - im) * h, (re + im) * h
        if sc == 1 and ss == -1: return (re + im) * h, (im - re) * h
        if sc == -1 and ss == 1: return (re + im) * (-h), (re - im) * h
        return (im - re) * h, (re + im) * (-h)
    return re * c - im * s, re * s + im * c

def _dft4(xs, sign):
    (a0, b0), (a1, b1), (a2, b2), (a3, b3) = xs
    sr, si = a0 + a2, b0 + b2
    dr, di = a0 - a2, b0 - b2
    tr, ti = a1 + a3, b1 + b3
    ur, ui = a1 - a3, b1 - b3
    if sign > 0:
        x1 = (dr - ui, di + ur); x3 = (dr + ui, di - ur)
    else:
        x1 = (dr + ui, di - ur); x3 = (dr - ui, di + ur)
    return [(sr + tr, si + ti), x1, (sr - tr, si - ti), x3]

def _fft16(xs, sign):
    t = [[None] * 4 for _ in range(4)]
    for b in range(4):
        y = _dft4([xs[4 * a + b] for a in range(4)], sign)
        for c in range(4):
            t[b][c] = _cmul_tw(y[c][0], y[c][1], b * c, sign)
    out = [None] * 16
    for c in range(4):
        y = _dft4([t[b][c] for b in range(4)], sign)
        for d in range(4):
            out[c + 4 * d] = y[d]
    return out

def make(order="B", bq=512, flags=None, oproj_bm=512, doA=True, doB=True):
    nq = S // bq
    sub = 128
    nsub = bq // sub
    XT = [(0, 128), (128, 128), (256, 128), (384, 64)]
    consts = _consts()

    def kern(ax_hbm, wr_hbm, wi_hbm, bx_hbm, c_hbm, wq_hbm, wuk_hbm, wuv_hbm, wo_hbm,
             ft_hbm, mf_hbm, mi_hbm, g_hbm, p_hbm, out_hbm,
             axT, wrT, wiT, ft, mf, mi, g, pm, rt, x1t, wp, y1, ys,
             x0, x1, x2, x3, c_s, wq_b, wuk_b, wuv_b,
             wq_s, wkv_s, q_all, k_s, v_s, out_s, xT, woT, sems, osem):
        xs = [x0, x1, x2, x3]
        dmas = {}
        n = [0]
        def dma(name, src, dst):
            cp = pltpu.make_async_copy(src, dst, sems.at[n[0]])
            n[0] += 1
            dmas[name] = cp
            cp.start()
        if doA:
            dma("ft", ft_hbm, ft)
            for t in range(4):
                dma(("ax", t), ax_hbm.at[:, pl.ds(512 * t, 512)], axT.at[:, pl.ds(512 * t, 512)])
            dma("pm", p_hbm, pm)
            dma("wr", wr_hbm, wrT)
            dma("wi", wi_hbm, wiT)
            dma("mf", mf_hbm, mf)
            dma("mi", mi_hbm, mi)
        dma("x", bx_hbm, xT)
        if doA:
            dma("g", g_hbm, g)
        for dt in range(2):
            dma(("wq", dt), wq_hbm.at[:, pl.ds(128 * dt, 128)], wq_b.at[dt])
        for t in range(8):
            dma(("c", t), c_hbm.at[:, pl.ds(128 * t, 128)], c_s.at[t])
        for dt in range(2):
            dma(("wuk", dt), wuk_hbm.at[:, pl.ds(128 * dt, 128)], wuk_b.at[dt])
        for dt in range(2):
            dma(("wuv", dt), wuv_hbm.at[:, pl.ds(128 * dt, 128)], wuv_b.at[dt])
        dma("wo", wo_hbm, woT)

        if doA:
            @pl.loop(0, 16)
            def _(k1):
                x1t[1, k1, 112:128, :] = jnp.zeros((16, 256), bf)
            @pl.loop(0, 16)
            def _(k1):
                wp[0, 1, k1] = jnp.zeros((128, 128), f32)
                wp[1, 1, k1] = jnp.zeros((128, 128), f32)
            dmas["ft"].wait()
            for t in range(4):
                dmas[("ax", t)].wait()
                cols = slice(512 * t, 512 * (t + 1))
                rt[:, cols] = jnp.dot(ft[...], axT[:, cols], preferred_element_type=f32)
            dmas["pm"].wait(); dmas["wr"].wait(); dmas["wi"].wait()
            @pl.loop(0, 16)
            def _(kt):
                cols = pl.ds(pl.multiple_of(kt * 128, 128), 128)
                k2 = pl.ds(pl.multiple_of(kt * 8, 8), 8)
                for a, wref in enumerate((wrT, wiT)):
                    r0 = lax.dot_general(pm[...], wref[0:128, cols], NT, preferred_element_type=f32)
                    r1 = lax.dot_general(pm[...], wref[128:DF, cols], NT, preferred_element_type=f32)
                    for k1 in range(16):
                        wp[a, 0, k1, k2, :] = r0[8 * k1:8 * k1 + 8]
                        wp[a, 1, k1, k2, 0:DF - 128] = r1[8 * k1:8 * k1 + 8]
            def fwd_fft(base_re, base_im, ftile):
                def body(gi, _):
                    r0 = pl.multiple_of(gi * 16, 16)
                    outs = [None] * 16
                    halves = []
                    for hf in range(2):
                        rr = pl.ds(base_re + r0 + 8 * hf, 8); ri = pl.ds(base_im + r0 + 8 * hf, 8)
                        zs = [(rt[rr, 128 * n1:128 * (n1 + 1)], rt[ri, 128 * n1:128 * (n1 + 1)]) for n1 in range(16)]
                        halves.append(_fft16(zs, -1))
                    for k1 in range(16):
                        for p in range(2):
                            v = jnp.concatenate([halves[0][k1][p], halves[1][k1][p]], axis=0).astype(bf)
                            x1t[ftile, k1, pl.ds(r0, 16), 128 * p:128 * (p + 1)] = v
                return body
            lax.fori_loop(0, 8, fwd_fft(0, 128, 0), None)
            lax.fori_loop(0, 7, fwd_fft(256, 368, 1), None)
            dmas["mf"].wait(); dmas["mi"].wait()
            @pl.loop(0, 16)
            def _(k1):
                for t in range(2):
                    x2 = lax.dot_general(mf[k1], x1t[t, k1], NT, preferred_element_type=f32)
                    xr, xi = x2[:128], x2[128:]
                    wr_, wi_ = wp[0, t, k1], wp[1, t, k1]
                    z = jnp.concatenate([xr * wr_ - xi * wi_, xr * wi_ + xi * wr_], axis=0).astype(bf)
                    y1[t, k1] = jnp.dot(mi[k1], z, preferred_element_type=f32)
            def inv_body(gi, _):
                r0 = pl.multiple_of(gi * 16, 16)
                for t in range(2):
                    halves = []
                    for hf in range(2):
                        rr = pl.ds(r0 + 8 * hf, 8); ri = pl.ds(128 + r0 + 8 * hf, 8)
                        zs = [(y1[t, k1, rr, :], y1[t, k1, ri, :]) for k1 in range(16)]
                        halves.append(_fft16(zs, 1))
                    for n1 in range(16):
                        for p in range(2):
                            v = jnp.concatenate([halves[0][n1][p], halves[1][n1][p]], axis=0).astype(bf)
                            ys[2 * p + t, pl.ds(128 * n1 + r0, 16), :] = v
            lax.fori_loop(0, 8, inv_body, None)
            dmas["g"].wait()
            @pl.loop(0, 4)
            def _(m):
                rows = pl.ds(pl.multiple_of(m * 512, 512), 512)
                a = jnp.concatenate([ys[t, rows, :] for t in range(4)], axis=1)
                out_s[rows, 0:448] = jnp.dot(a, g[...], preferred_element_type=f32).astype(bf)

        dmas["x"].wait()
        for t, (o, w) in enumerate(XT):
            @pl.loop(0, S // 128)
            def _(sb):
                rows = pl.ds(pl.multiple_of(sb * 128, 128), 128)
                xs[t][rows, :] = xT[o:o+w, rows].T
        for dt in range(2): dmas[("wq", dt)].wait()
        wq_i = wq_b.bitcast(jnp.int32)

        def extract_q(j, slot):
            for dt in range(2):
                u = wq_i.at[dt, pl.ds(j, M * 8 - 7)][pl.ds(0, M, stride=8), :]
                lo = pltpu.bitcast(u << 16, f32).astype(bf)
                hi = pltpu.bitcast(u & jnp.int32(-65536), f32).astype(bf)
                wq_s[slot, dt] = lo
                wq_s[slot, 2 + dt] = hi
        extract_q(0, 0)
        def qbody(j, _):
            slot = j % 2
            w = jnp.concatenate([wq_s[slot, t] for t in range(4)], axis=1)
            for m in range(4):
                rows = slice(m * 512, (m + 1) * 512)
                xr = jnp.concatenate([xs[t][rows, :] for t in range(4)], axis=1)
                r = (jnp.dot(xr, w, preferred_element_type=f32) * QSCALE).astype(bf)
                for t in range(4):
                    q_all[4 * j + t, rows, :] = r[:, t * 128:(t + 1) * 128]
            extract_q(jnp.minimum(j + 1, 7), 1 - slot)
        lax.fori_loop(0, 8, qbody, None)

        for t in range(8): dmas[("c", t)].wait()
        for dt in range(2): dmas[("wuk", dt)].wait(); dmas[("wuv", dt)].wait()
        wuk_i = wuk_b.bitcast(jnp.int32)
        wuv_i = wuv_b.bitcast(jnp.int32)
        def extract_kv(h, slot):
            j = h // 2
            sh = (1 - h % 2) * 16
            for a, wi in enumerate((wuk_i, wuv_i)):
                for dt in range(2):
                    u = wi.at[dt, pl.ds(j, DC * 8 - 7)][pl.ds(0, DC, stride=8), :]
                    wkv_s[slot, 2 * a + dt] = pltpu.bitcast((u << sh) & jnp.int32(-65536), f32).astype(bf)
        extract_kv(0, 0)

        row = lax.broadcasted_iota(jnp.int32, (sub, sub), 0)
        col = lax.broadcasted_iota(jnp.int32, (sub, sub), 1)
        tri = col <= row

        def hbody(h, _):
            slot = h % 2
            st = {}
            def qload(r0, r1):
                return jnp.concatenate([q_all[2 * h, r0:r1, :], q_all[2 * h + 1, r0:r1, :]], axis=1)
            def kload(r0, r1):
                return jnp.concatenate([k_s[0, r0:r1, :], k_s[1, r0:r1, :]], axis=1)
            def vload(r0, r1):
                return jnp.concatenate([v_s[0, r0:r1, :], v_s[1, r0:r1, :]], axis=1)
            def kv(m):
                rows = slice(m * 512, (m + 1) * 512)
                cr = jnp.concatenate([c_s[t, rows, :] for t in range(8)], axis=1)
                w = jnp.concatenate([wkv_s[slot, t] for t in range(4)], axis=1)
                r = jnp.dot(cr, w, preferred_element_type=f32).astype(bf)
                for t in range(2):
                    k_s[t, rows, :] = r[:, t * 128:(t + 1) * 128]
                    v_s[t, rows, :] = r[:, 256 + t * 128:256 + (t + 1) * 128]
            def qk(i, j):
                if j < i:
                    s = lax.dot_general(qload(i*bq, (i+1)*bq), kload(j*bq, (j+1)*bq), NT, preferred_element_type=f32)
                    st[("s", i, j)] = s
                    mj = jnp.max(s, axis=1, keepdims=True)
                else:
                    parts = [[] for _ in range(nsub)]
                    for t in range(nsub):
                        r0 = t * sub
                        s = lax.dot_general(qload(i*bq + r0, (i+1)*bq), kload(j*bq + r0, j*bq + r0 + sub), NT, preferred_element_type=f32)
                        parts[t].append(jnp.where(tri, s[:sub], NEG))
                        for r in range(t + 1, nsub):
                            parts[r].append(s[(r-t)*sub:(r-t+1)*sub])
                    st[("sd", i)] = parts
                    ms = [jnp.max(functools.reduce(jnp.maximum, parts[r]), axis=1, keepdims=True) for r in range(nsub)]
                    mj = jnp.concatenate(ms, axis=0)
                st[("m", i)] = mj if ("m", i) not in st else jnp.maximum(st[("m", i)], mj)
            def pv(i, j):
                m = st[("m", i)]
                if j < i:
                    p = jnp.exp2(st.pop(("s", i, j)) - m)
                    lj = functools.reduce(jnp.add, [p[:, t*sub:(t+1)*sub] for t in range(nsub)])
                    o = jnp.dot(p.astype(bf), vload(j*bq, (j+1)*bq), preferred_element_type=f32)
                    st[("l", i)] = lj if ("l", i) not in st else st[("l", i)] + lj
                    st[("o", i)] = o if ("o", i) not in st else st[("o", i)] + o
                else:
                    parts = st.pop(("sd", i))
                    for r in range(nsub):
                        rows = slice(r*sub, (r+1)*sub)
                        w = (r+1)*sub
                        ps = [jnp.exp2(x - m[rows]) for x in parts[r]]
                        lj = functools.reduce(jnp.add, ps)
                        p = jnp.concatenate(ps, axis=1) if r > 0 else ps[0]
                        o = jnp.dot(p.astype(bf), vload(j*bq, j*bq + w), preferred_element_type=f32)
                        if ("l", i) in st:
                            lj = lj + st[("l", i)][rows]; o = o + st[("o", i)][rows]
                        l = jnp.sum(lj, axis=1, keepdims=True)
                        rl = pl.reciprocal(l, approx=True)
                        rl = rl * (2.0 - l * rl)
                        ctx = (o * rl).astype(bf)
                        rr = slice(i*bq + r*sub, i*bq + (r+1)*sub)
                        q_all[2 * h, rr, :] = ctx[:, :128]
                        q_all[2 * h + 1, rr, :] = ctx[:, 128:]
            seq = []
            if order == "A":
                for i in range(nq + 1):
                    if i < nq: seq.append(("kv", i))
                    a = [("qk", i, j) for j in range(i+1)] if i < nq else []
                    b = [("pv", i-1, j) for j in range(i)] if i > 0 else []
                    for t in range(max(len(a), len(b))):
                        if t < len(a): seq.append(a[t])
                        if t < len(b): seq.append(b[t])
                    if i == 1: seq.append(("ex",))
            elif order == "B":
                seq += [("kv", i) for i in range(nq)] + [("ex",)]
                for i in range(nq + 1):
                    a = [("qk", i, j) for j in range(i+1)] if i < nq else []
                    b = [("pv", i-1, j) for j in range(i)] if i > 0 else []
                    for t in range(max(len(a), len(b))):
                        if t < len(a): seq.append(a[t])
                        if t < len(b): seq.append(b[t])
            else:
                seq = order
            for op in seq:
                if op[0] == "kv": kv(op[1])
                elif op[0] == "qk": qk(*op[1:])
                elif op[0] == "pv": pv(*op[1:])
                elif op[0] == "ex": extract_kv(jnp.minimum(h + 1, H - 1), 1 - slot)
        lax.fori_loop(0, H, hbody, None)

        dmas["wo"].wait()
        def obody(m, _):
            rows = pl.ds(pl.multiple_of(m * oproj_bm, oproj_bm), oproj_bm)
            acc = None
            for kk in range(8):
                a = jnp.concatenate([q_all[4 * kk + t, rows, :] for t in range(4)], axis=1)
                w = jnp.concatenate([woT[2*kk], woT[2*kk+1]], axis=1)
                r = lax.dot_general(a, w, NT, preferred_element_type=f32)
                acc = r if acc is None else acc + r
            out_s[rows, 448:896] = acc.astype(bf)
            if not doA:
                out_s[rows, 0:448] = jnp.zeros((oproj_bm, 448), bf)
            pltpu.make_async_copy(out_s.at[rows], out_hbm.at[rows], osem.at[m]).start()
        lax.fori_loop(0, S // oproj_bm, obody, None)
        def owait(m, _):
            rows = pl.ds(pl.multiple_of(m * oproj_bm, oproj_bm), oproj_bm)
            pltpu.make_async_copy(out_s.at[rows], out_hbm.at[rows], osem.at[m]).wait()
        lax.fori_loop(0, S // oproj_bm, owait, None)

    def fn(A_x, A_w_r, A_w_i, B_x, B_c_kv, B_w_q, B_w_uk, B_w_uv, B_w_o):
        V = pltpu.VMEM
        scratch = ([V((M, S), bf), V((DF, S), bf), V((DF, S), bf), V((480, M), bf), V((16, 256, 256), bf), V((16, 256, 256), bf),
                    V((512, M), bf), V((128, 128), bf), V((480, S), f32), V((2, 16, 128, 256), bf), V((2, 2, 16, 128, 128), f32),
                    V((2, 16, 256, 128), f32), V((4, S, 128), bf)]
            + [V((S, w), bf) for _, w in XT] + [V((8, S, 128), bf), V((2, M*H, 128), bf), V((2, DC*H, 128), bf), V((2, DC*H, 128), bf)]
            + [V((2, 4, M, 128), bf), V((2, 4, DC, 128), bf), V((32, S, 128), bf), V((2, S, 128), bf), V((2, S, 128), bf), V((S, 896), bf),
               V((M, S), bf), V((H, M, D), bf),
               pltpu.SemaphoreType.DMA((32,)), pltpu.SemaphoreType.DMA((16,))])
        out = pl.pallas_call(kern, in_specs=[pl.BlockSpec(memory_space=pl.ANY)]*14, out_specs=pl.BlockSpec(memory_space=pl.ANY),
            out_shape=jax.ShapeDtypeStruct((S, 896), bf), scratch_shapes=scratch,
            compiler_params=pltpu.CompilerParams(vmem_limit_bytes=120<<20, flags=flags))(
            A_x.reshape(S, M).T, A_w_r.T, A_w_i.T, B_x.reshape(S, M).T, B_c_kv.reshape(S, DC), B_w_q.reshape(M*H, D),
            B_w_uk.reshape(DC*H, D), B_w_uv.reshape(DC*H, D), B_w_o.transpose(0, 2, 1), *consts)
        return out.reshape(1, S, 896)
    return fn


@jax.jit
def pallas_concat_heads__spectral_gfnet__compressed_kv_cla__prompt_kernel(
    A_x, A_w_r, A_w_i, B_x, B_c_kv, B_w_q, B_w_uk, B_w_uv, B_w_o,
):
    return make()(A_x, A_w_r, A_w_i, B_x, B_c_kv, B_w_q, B_w_uk, B_w_uv, B_w_o)
```

```python
import functools, math, contextlib
import numpy as np, jax, jax.numpy as jnp
import ml_dtypes
from jax import lax
from jax.experimental import pallas as pl
from jax.experimental.pallas import tpu as pltpu

S, M, H, D, DC = 2048, 448, 16, 256, 1024
DF = M // 2 + 1
HM = M // 2
f32, bf = jnp.float32, jnp.bfloat16
NT = (((1,), (1,)), ((), ()))
LOG2E = 1.4426950408889634
QSCALE = (D ** -0.5) * LOG2E
NEG = -1e9 * LOG2E

def _consts():
    nb = ml_dtypes.bfloat16
    d = np.arange(M, dtype=np.float64)
    f = np.arange(DF, dtype=np.float64)
    ang = 2 * np.pi * ((f[:, None] * d[None, :]) % M) / M
    cs, sn = np.cos(ang), np.sin(ang)
    FT = np.zeros((480, M))
    FT[0:128] = cs[:128]; FT[128:256] = -sn[:128]
    FT[256:256 + 97] = cs[128:]; FT[368:368 + 97] = -sn[128:]
    k1 = np.arange(16)[:, None, None]; k2 = np.arange(128)[None, :, None]; n2 = np.arange(128)[None, None, :]
    a = 2 * np.pi * ((n2 * (k1 + 16 * k2)) % S) / S
    Mr, Mi = np.cos(a), -np.sin(a)
    MF = np.concatenate([np.concatenate([Mr, -Mi], 2), np.concatenate([Mi, Mr], 2)], 1)
    MI = np.transpose(MF, (0, 2, 1)) / S
    c = np.full(DF, 2.0); c[0] = 1.0; c[-1] = 1.0
    Gc = (c[:, None] * cs) / M; Gs = -(c[:, None] * sn) / M
    G = np.zeros((512, M))
    G[0:128] = Gc[:128]; G[128:225] = Gc[128:]; G[256:384] = Gs[:128]; G[384:481] = Gs[128:]
    G = np.ascontiguousarray(G.T)
    P = np.zeros((128, 128))
    for a_ in range(16):
        for j in range(8):
            P[a_ * 8 + j, 16 * j + a_] = 1.0
    return tuple(np.asarray(x, dtype=np.float32).astype(nb) for x in (FT, MF, MI, G, P))

_C = [math.cos(2 * math.pi * k / 16) for k in range(16)]
_S = [math.sin(2 * math.pi * k / 16) for k in range(16)]

def _cmul_tw(re, im, k, sign):
    k = k % 16
    c, s = _C[k], sign * _S[k]
    if k == 0: return re, im
    if k == 4: return (-sign * im, sign * re) if True else None
    if k == 8: return -re, -im
    if k == 12: return (sign * im, -sign * re)
    if k in (2, 6, 10, 14):
        h = math.sqrt(0.5)
        sc, ss = (1 if c > 0 else -1), (1 if s > 0 else -1)
        a = (re - im) if sc == ss else (re + im)
        b = (re + im) if sc == ss else (re - im)
        if sc == 1 and ss == 1: return (re - im) * h, (re + im) * h
        if sc == 1 and ss == -1: return (re + im) * h, (im - re) * h
        if sc == -1 and ss == 1: return (re + im) * (-h), (re - im) * h
        return (im - re) * h, (re + im) * (-h)
    return re * c - im * s, re * s + im * c

def _dft4(xs, sign):
    (a0, b0), (a1, b1), (a2, b2), (a3, b3) = xs
    sr, si = a0 + a2, b0 + b2
    dr, di = a0 - a2, b0 - b2
    tr, ti = a1 + a3, b1 + b3
    ur, ui = a1 - a3, b1 - b3
    if sign > 0:
        x1 = (dr - ui, di + ur); x3 = (dr + ui, di - ur)
    else:
        x1 = (dr + ui, di - ur); x3 = (dr - ui, di + ur)
    return [(sr + tr, si + ti), x1, (sr - tr, si - ti), x3]

def _fft16(xs, sign):
    t = [[None] * 4 for _ in range(4)]
    for b in range(4):
        y = _dft4([xs[4 * a + b] for a in range(4)], sign)
        for c in range(4):
            t[b][c] = _cmul_tw(y[c][0], y[c][1], b * c, sign)
    out = [None] * 16
    for c in range(4):
        y = _dft4([t[b][c] for b in range(4)], sign)
        for d in range(4):
            out[c + 4 * d] = y[d]
    return out

SCOPES = False
_cur = [None]
def mark(name):
    if not SCOPES: return
    if _cur[0] is not None:
        _cur[0].__exit__(None, None, None); _cur[0] = None
    if name is not None:
        _cur[0] = jax.named_scope(name); _cur[0].__enter__()

_SP = {1: ((11, 1), (22, 1)), 2: ((21, 1), (22, -1)), 3: ((12, 1), (22, 1)), 4: ((11, 1), (21, 1)),
       5: ((11, -1), (12, 1)), 6: ((22, 1),), 7: ((11, 1),)}
_CNT = {11: 4, 12: 2, 21: 2, 22: 4}

def make(order="S4", sbm=512, qbm=512, sorder=(1,2,3,4,5,6,7), bq=512, flags=None, oproj_bm=512, doA=True, doB=True, dft_unroll=4, wp_unroll=4, when=dict(c='qproj',wuk='qproj',wuv='qproj',wo='kvpre',g='kvpre'), pv_split=256):
    nq = S // bq
    sub = 128
    nsub = bq // sub
    XT = [(0, 128), (128, 128), (256, 128), (384, 64)]
    consts = _consts()

    def kern(ax_hbm, wr_hbm, wi_hbm, bx_hbm, c_hbm, wq_hbm, wuk_hbm, wuv_hbm, wo_hbm,
             ft_hbm, mf_hbm, mi_hbm, g_hbm, p_hbm, out_hbm,
             axT, wrT, wiT, ft, mf, mi, g, pm, rt, x1t, wp, y1, ys,
             x0, x1, c_s, wq_b, wuk_b, wuv_b,
             wq_s, wkv_s, q_all, k_s, v_s, out_s, xT, woT, pc, sems, osem):
        dmas = {}
        n = [0]
        def dma(name, src, dst):
            cp = pltpu.make_async_copy(src, dst, sems.at[n[0]])
            n[0] += 1
            dmas[name] = cp
        dma("ft", ft_hbm, ft)
        for t in range(4):
            dma(("ax", t), ax_hbm.at[:, pl.ds(512 * t, 512)], axT.at[:, pl.ds(512 * t, 512)])
        dma("pm", p_hbm, pm)
        dma("wr", wr_hbm, wrT)
        dma("wi", wi_hbm, wiT)
        dma("x", bx_hbm, xT)
        for t in range(4):
            dma(("mf", t), mf_hbm.at[pl.ds(4 * t, 4)], mf.at[pl.ds(4 * t, 4)])
            dma(("mi", t), mi_hbm.at[pl.ds(4 * t, 4)], mi.at[pl.ds(4 * t, 4)])
        for dt in range(2):
            dma(("wq", dt), wq_hbm.at[:, pl.ds(128 * dt, 128)], wq_b.at[dt])
        for t in range(8):
            dma(("c", t), c_hbm.at[:, pl.ds(128 * t, 128)], c_s.at[t])
        for dt in range(2):
            dma(("wuk", dt), wuk_hbm.at[:, pl.ds(128 * dt, 128)], wuk_b.at[dt])
        for dt in range(2):
            dma(("wuv", dt), wuv_hbm.at[:, pl.ds(128 * dt, 128)], wuv_b.at[dt])
        dma("g", g_hbm, g)
        dma("wo", wo_hbm, woT)
        started = set()
        def start(point):
            for name in dmas:
                key = name[0] if isinstance(name, tuple) else name
                if when.get(key, "begin") == point:
                    dmas[name].start(); started.add(name)
        start("begin")

        if doA:
            mark('A_zero')
            @pl.loop(0, 16)
            def _(k1):
                x1t[1, k1, 112:128, :] = jnp.zeros((16, 256), bf)
            @pl.loop(0, 16)
            def _(k1):
                wp[0, 1, k1] = jnp.zeros((128, 128), f32)
                wp[1, 1, k1] = jnp.zeros((128, 128), f32)
            mark('A_dfwd'); start('A_dfwd')
            dmas["ft"].wait()
            for t in range(4):
                dmas[("ax", t)].wait()
                cols = slice(512 * t, 512 * (t + 1))
                rt[:, cols] = jnp.dot(ft[...], axT[:, cols], preferred_element_type=f32)
            mark('A_wperm'); start('A_wperm')
            dmas["pm"].wait(); dmas["wr"].wait(); dmas["wi"].wait()
            def wperm(kt, cols, k2):
                for a, wref in enumerate((wrT, wiT)):
                    r = lax.dot_general(pm[...], wref[:, cols], NT, preferred_element_type=f32)
                    for k1 in range(16):
                        wp[a, 0, k1, k2, :] = r[8 * k1:8 * k1 + 8, :128]
                        wp[a, 1, k1, k2, 0:DF - 128] = r[8 * k1:8 * k1 + 8, 128:]
            def fwd_fft(base_re, base_im, ftile, r0):
                halves = []
                for hf in range(2):
                    rr = pl.ds(base_re + r0 + 8 * hf, 8); ri = pl.ds(base_im + r0 + 8 * hf, 8)
                    zs = [(rt[rr, 128 * n1:128 * (n1 + 1)], rt[ri, 128 * n1:128 * (n1 + 1)]) for n1 in range(16)]
                    halves.append(_fft16(zs, -1))
                for k1 in range(16):
                    for p in range(2):
                        v = jnp.concatenate([halves[0][k1][p], halves[1][k1][p]], axis=0).astype(bf)
                        x1t[ftile, k1, pl.ds(r0, 16), 128 * p:128 * (p + 1)] = v
            @pl.loop(0, 8)
            def _(gi):
                for u in range(2):
                    kt = gi * 2 + u
                    wperm(kt, pl.ds(pl.multiple_of(kt * 128, 128), 128), pl.ds(pl.multiple_of(kt * 8, 8), 8))
                fwd_fft(0, 128, 0, pl.multiple_of(gi * 16, 16))
                fwd_fft(256, 368, 1, pl.multiple_of(jnp.minimum(gi, 6) * 16, 16))
            mark('A_dft128'); start('A_dft128')
            dmas["x"].wait()
            def d1(k1):
                xt = jnp.concatenate([x1t[0, k1], x1t[1, k1]], axis=0)
                return lax.dot_general(mf[k1], xt, NT, preferred_element_type=f32)
            def d2(k1, x2):
                xr, xi = x2[:128], x2[128:]
                wr_ = jnp.concatenate([wp[0, 0, k1], wp[0, 1, k1]], axis=1)
                wi_ = jnp.concatenate([wp[1, 0, k1], wp[1, 1, k1]], axis=1)
                z = jnp.concatenate([xr * wr_ - xi * wi_, xr * wi_ + xi * wr_], axis=0).astype(bf)
                y = jnp.dot(mi[k1], z, preferred_element_type=f32)
                y1[0, k1] = y[:, :128]
                y1[1, k1] = y[:, 128:]
            if dft_unroll == 16:
                for kb in range(4):
                    dmas[("mf", kb)].wait(); dmas[("mi", kb)].wait()
                    x2s = [d1(kb * 4 + u) for u in range(4)]
                    for u in range(4):
                        d2(kb * 4 + u, x2s[u])
                    for t, (o, w) in enumerate(XT):
                        for sb in range(4):
                            rr = slice(kb * 512 + sb * 128, kb * 512 + (sb + 1) * 128)
                            xs[t][rr, :] = xT[o:o+w, rr].T
            else:
                sem_mf = list(dmas).index(("mf", 0))
                @pl.loop(0, 4)
                def _(kb):
                    blk = pl.ds(4 * kb, 4)
                    pltpu.make_async_copy(mf_hbm.at[blk], mf.at[blk], sems.at[sem_mf + 2 * kb]).wait()
                    pltpu.make_async_copy(mi_hbm.at[blk], mi.at[blk], sems.at[sem_mf + 2 * kb + 1]).wait()
                    x2s = [d1(kb * 4 + u) for u in range(4)]
                    for u in range(4):
                        d2(kb * 4 + u, x2s[u])
                    for sb in range(2):
                        c0 = pl.multiple_of(kb * 256 + sb * 128, 128)
                        lo = pl.ds(c0, 128); hi = pl.ds(S // 2 + c0, 128)
                        a11 = xT[0:HM, lo].astype(f32); a12 = xT[HM:M, lo].astype(f32)
                        a21 = xT[0:HM, hi].astype(f32); a22 = xT[HM:M, hi].astype(f32)
                        for i, pv_ in enumerate((a11 + a22, a21 + a22, a11, a22, a11 + a12, a21 - a11, a12 - a22)):
                            x0[i, lo, :] = pv_[0:128].T.astype(bf)
                            x1[i, lo, :] = pv_[128:HM].T.astype(bf)

        mark('qproj'); start('qproj')
        dmas[("wq", 0)].wait()
        wq_i = wq_b.bitcast(jnp.int32)
        def inv_fft(r0):
            for t in range(2):
                halves = []
                for hf in range(2):
                    rr = pl.ds(r0 + 8 * hf, 8); ri = pl.ds(128 + r0 + 8 * hf, 8)
                    zs = [(y1[t, k1, rr, :], y1[t, k1, ri, :]) for k1 in range(16)]
                    halves.append(_fft16(zs, 1))
                for n1 in range(16):
                    for p in range(2):
                        v = jnp.concatenate([halves[0][n1][p], halves[1][n1][p]], axis=0).astype(bf)
                        ys[2 * p + t, pl.ds(128 * n1 + r0, 16), :] = v
        def extract_q(it):
            dt = it // 4
            for pb in range(2):
                p = 2 * (it % 4) + pb
                u = wq_i.at[dt, pl.ds(p, M * 8 - 7)][pl.ds(0, M, stride=8), :]
                lo = pltpu.bitcast(u << 16, f32)
                hi = pltpu.bitcast(u & jnp.int32(-65536), f32)
                b11, b12, b21, b22 = lo[:HM], hi[:HM], lo[HM:], hi[HM:]
                for i, qv in enumerate((b11 + b22, b11, b12 - b22, b21 - b11, b22, b11 + b12, b21 + b22)):
                    wq_s[i, pb] = qv.astype(bf)
        extract_q(0)
        def qbody(it, _):
            @pl.when(it == 3)
            def _():
                dmas[("wq", 1)].wait()
            dt = it // 4
            h0 = 4 * (it % 4)
            st = {}
            for ch in range(S // 2 // qbm):
                for i in sorder:
                    rows = slice(ch * qbm, (ch + 1) * qbm)
                    lhs = jnp.concatenate([x0[i - 1, rows, :], x1[i - 1, rows, :]], axis=1)
                    w = jnp.concatenate([wq_s[i - 1, 0], wq_s[i - 1, 1]], axis=1)
                    m = jnp.dot(lhs, w, preferred_element_type=f32)
                    for blk, sign in _SP[i]:
                        key = (blk, ch)
                        if key not in st:
                            st[key] = [m if sign > 0 else -m, 1]
                        else:
                            st[key][0] = st[key][0] + m if sign > 0 else st[key][0] - m
                            st[key][1] += 1
                        if st[key][1] == _CNT[blk]:
                            r = (st.pop(key)[0] * QSCALE).astype(bf)
                            base = (blk // 10 - 1) * (S // 2) + ch * qbm
                            hh = h0 + (blk % 10 - 1)
                            q_all[2 * hh + dt, base:base + qbm, :] = r[:, :128]
                            q_all[2 * (hh + 2) + dt, base:base + qbm, :] = r[:, 128:]
            extract_q(jnp.minimum(it + 1, 7))
            inv_fft(pl.multiple_of(it * 16, 16))
        lax.fori_loop(0, 8, qbody, None)

        mark('kvpre'); start('kvpre')
        for t in range(8): dmas[("c", t)].wait()
        for dt in range(2): dmas[("wuk", dt)].wait(); dmas[("wuv", dt)].wait()
        wuk_i = wuk_b.bitcast(jnp.int32)
        wuv_i = wuv_b.bitcast(jnp.int32)
        HK = DC // 2
        def extract_kv(h):
            j = h // 2
            sh = (1 - h % 2) * 16
            for a, wi in enumerate((wuk_i, wuv_i)):
                b = {}
                for dt in range(2):
                    u = wi.at[dt, pl.ds(j, DC * 8 - 7)][pl.ds(0, DC, stride=8), :]
                    w = pltpu.bitcast((u << sh) & jnp.int32(-65536), f32)
                    b[(0, dt)] = w[:HK]; b[(1, dt)] = w[HK:]
                b11, b12, b21, b22 = b[(0, 0)], b[(0, 1)], b[(1, 0)], b[(1, 1)]
                for i, qv in enumerate((b11 + b22, b11, b12 - b22, b21 - b11, b22, b11 + b12, b21 + b22)):
                    wkv_s[i, a] = qv.astype(bf)
        extract_kv(0)
        HS = S // 2
        @pl.loop(0, HS // 128)
        def _(gi):
            r0 = pl.multiple_of(gi * 128, 128)
            top = pl.ds(r0, 128); bot = pl.ds(HS + r0, 128)
            for t in range(4):
                a11 = c_s[t, top, :].astype(f32); a12 = c_s[4 + t, top, :].astype(f32)
                a21 = c_s[t, bot, :].astype(f32); a22 = c_s[4 + t, bot, :].astype(f32)
                for i, pv_ in enumerate((a11 + a22, a21 + a22, a11 + a12, a21 - a11, a12 - a22)):
                    pc[i, t, top, :] = pv_.astype(bf)

        row = lax.broadcasted_iota(jnp.int32, (sub, sub), 0)
        col = lax.broadcasted_iota(jnp.int32, (sub, sub), 1)
        tri = col <= row

        def hbody(h, _):
            st = {}
            def qload(r0, r1):
                return jnp.concatenate([q_all[2 * h, r0:r1, :], q_all[2 * h + 1, r0:r1, :]], axis=1)
            def kload(r0, r1):
                return jnp.concatenate([k_s[0, r0:r1, :], k_s[1, r0:r1, :]], axis=1)
            def vload(r0, r1):
                return jnp.concatenate([v_s[0, r0:r1, :], v_s[1, r0:r1, :]], axis=1)
            def sp(i, ch):
                rows = slice(ch * sbm, (ch + 1) * sbm)
                if i == 3:
                    lhs = [c_s[t, rows, :] for t in range(4)]
                elif i == 4:
                    lhs = [c_s[4 + t, HS + ch * sbm:HS + (ch + 1) * sbm, :] for t in range(4)]
                else:
                    pi = {1: 0, 2: 1, 5: 2, 6: 3, 7: 4}[i]
                    lhs = [pc[pi, t, rows, :] for t in range(4)]
                w = jnp.concatenate([wkv_s[i - 1, 0], wkv_s[i - 1, 1]], axis=1)
                m = jnp.dot(jnp.concatenate(lhs, axis=1), w, preferred_element_type=f32)
                for blk, sign in {1: ((11, 1), (22, 1)), 2: ((21, 1), (22, -1)), 3: ((12, 1), (22, 1)), 4: ((11, 1), (21, 1)),
                                  5: ((11, -1), (12, 1)), 6: ((22, 1),), 7: ((11, 1),)}[i]:
                    key = ("c", blk, ch)
                    if key not in st:
                        st[key] = [m if sign > 0 else -m, 1]
                    else:
                        st[key][0] = st[key][0] + m if sign > 0 else st[key][0] - m
                        st[key][1] += 1
                    if st[key][1] == {11: 4, 12: 2, 21: 2, 22: 4}[blk]:
                        r = st.pop(key)[0].astype(bf)
                        base = (blk // 10 - 1) * HS + ch * sbm
                        dt = blk % 10 - 1
                        k_s[dt, base:base + sbm, :] = r[:, :128]
                        v_s[dt, base:base + sbm, :] = r[:, 128:]
            def qk(i, j):
                if j < i:
                    s = lax.dot_general(qload(i*bq, (i+1)*bq), kload(j*bq, (j+1)*bq), NT, preferred_element_type=f32)
                    st[("s", i, j)] = s
                    mj = jnp.max(s, axis=1, keepdims=True)
                else:
                    parts = [[] for _ in range(nsub)]
                    for t in range(nsub):
                        r0 = t * sub
                        s = lax.dot_general(qload(i*bq + r0, (i+1)*bq), kload(j*bq + r0, j*bq + r0 + sub), NT, preferred_element_type=f32)
                        parts[t].append(jnp.where(tri, s[:sub], NEG))
                        for r in range(t + 1, nsub):
                            parts[r].append(s[(r-t)*sub:(r-t+1)*sub])
                    st[("sd", i)] = parts
                    ms = [jnp.max(functools.reduce(jnp.maximum, parts[r]), axis=1, keepdims=True) for r in range(nsub)]
                    mj = jnp.concatenate(ms, axis=0)
                st[("m", i)] = mj if ("m", i) not in st else jnp.maximum(st[("m", i)], mj)
            def pv(i, j):
                m = st[("m", i)]
                if j < i:
                    sfull = st.pop(("s", i, j))
                    for c0 in range(0, bq, pv_split):
                        p = jnp.exp2(sfull[:, c0:c0 + pv_split] - m)
                        lj = functools.reduce(jnp.add, [p[:, t*sub:(t+1)*sub] for t in range(pv_split // sub)])
                        o = jnp.dot(p.astype(bf), vload(j*bq + c0, j*bq + c0 + pv_split), preferred_element_type=f32)
                        st[("l", i)] = lj if ("l", i) not in st else st[("l", i)] + lj
                        st[("o", i)] = o if ("o", i) not in st else st[("o", i)] + o
                else:
                    parts = st.pop(("sd", i))
                    for r in range(nsub):
                        rows = slice(r*sub, (r+1)*sub)
                        w = (r+1)*sub
                        ps = [jnp.exp2(x - m[rows]) for x in parts[r]]
                        lj = functools.reduce(jnp.add, ps)
                        p = jnp.concatenate(ps, axis=1) if r > 0 else ps[0]
                        o = jnp.dot(p.astype(bf), vload(j*bq, j*bq + w), preferred_element_type=f32)
                        if ("l", i) in st:
                            lj = lj + st[("l", i)][rows]; o = o + st[("o", i)][rows]
                        l = jnp.sum(lj, axis=1, keepdims=True)
                        rl = pl.reciprocal(l, approx=True)
                        rl = rl * (2.0 - l * rl)
                        ctx = (o * rl).astype(bf)
                        rr = slice(i*bq + r*sub, i*bq + (r+1)*sub)
                        q_all[2 * h, rr, :] = ctx[:, :128]
                        q_all[2 * h + 1, rr, :] = ctx[:, 128:]
            att = []
            for i in range(nq - 2, -2, -1):
                a = [("qk", i, j) for j in range(i+1)] if i >= 0 else []
                b = [("pv", i+1, j) for j in range(i+2)]
                for t in range(max(len(a), len(b))):
                    if t < len(a): att.append(a[t])
                    if t < len(b): att.append(b[t])
            P = sorder
            if order == "S1":
                seq = [("sp", i, 0) for i in P] + [("qk", 3, 0)] + [("sp", i, 1) for i in P[:3]] + [("qk", 3, 2)] + [("sp", i, 1) for i in P[3:]] + [("qk", 3, 1), ("qk", 3, 3), ("ex",)] + att
            elif order == "S2":
                seq = [("sp", i, 0) for i in P] + [("sp", i, 1) for i in P] + [("qk", 3, j) for j in range(4)] + [("ex",)] + att
            elif order == "S3":
                seq = [("sp", i, 0) for i in P] + [("sp", i, 1) for i in P] + [("ex",)] + [("qk", 3, j) for j in range(4)] + att
            elif order == "S4":
                seq = [("sp", i, 0) for i in P] + [("qk", 3, 0), ("qk", 3, 2)] + [("sp", i, 1) for i in P] + [("qk", 3, 1), ("qk", 3, 3), ("ex",)] + att
            else:
                seq = order
            if sbm == 1024:
                seq = [("sp", i, 0) for i in P] + [("qk", 3, j) for j in range(4)] + [("ex",)] + att
            for op in seq:
                if op[0] == "sp": sp(*op[1:])
                elif op[0] == "qk": qk(*op[1:])
                elif op[0] == "pv": pv(*op[1:])
                elif op[0] == "ex": extract_kv(jnp.minimum(h + 1, H - 1))
        lax.fori_loop(0, H, hbody, None)

        mark('oproj'); start('oproj')
        dmas["wo"].wait(); dmas["g"].wait()
        nt_per = oproj_bm // 128
        def obody(m, _):
            for u in range(nt_per):
                r0 = pl.multiple_of(m * oproj_bm + u * 128, 128)
                rows = pl.ds(r0, 128)
                y = jnp.concatenate([ys[t, rows, :] for t in range(4)], axis=1)
                at = lax.dot_general(g[...], y, NT, preferred_element_type=f32)
                ctx = jnp.concatenate([q_all[t, rows, :] for t in range(32)], axis=1)
                w = jnp.concatenate([woT[hh] for hh in range(H)], axis=1)
                bt = lax.dot_general(w, ctx, NT, preferred_element_type=f32)
                tt = jnp.concatenate([at, bt], axis=0)
                for c in range(7):
                    out_s[rows, c * 128:(c + 1) * 128] = tt[c * 128:(c + 1) * 128].T.astype(bf)
                pltpu.make_async_copy(out_s.at[rows], out_hbm.at[rows], osem.at[m * nt_per + u]).start()
        lax.fori_loop(0, S // oproj_bm, obody, None)
        mark('owait')
        def owait(m, _):
            rows = pl.ds(pl.multiple_of(m * 128, 128), 128)
            pltpu.make_async_copy(out_s.at[rows], out_hbm.at[rows], osem.at[m]).wait()
        lax.fori_loop(0, S // 128, owait, None)
        mark(None)

    def fn(A_x, A_w_r, A_w_i, B_x, B_c_kv, B_w_q, B_w_uk, B_w_uv, B_w_o):
        V = pltpu.VMEM
        scratch = ([V((M, S), bf), V((DF, S), bf), V((DF, S), bf), V((480, M), bf), V((16, 256, 256), bf), V((16, 256, 256), bf),
                    V((M, 512), bf), V((128, 128), bf), V((480, S), f32), V((2, 16, 128, 256), bf), V((2, 2, 16, 128, 128), f32),
                    V((2, 16, 256, 128), f32), V((4, S, 128), bf)]
            + [V((7, S // 2, 128), bf), V((7, S // 2, HM - 128), bf)] + [V((8, S, 128), bf), V((2, M*H, 128), bf), V((2, DC*H, 128), bf), V((2, DC*H, 128), bf)]
            + [V((7, 2, HM, 128), bf), V((7, 2, DC // 2, 128), bf), V((32, S, 128), bf), V((2, S, 128), bf), V((2, S, 128), bf), V((S, 896), bf),
               V((M, S), bf), V((H, M, D), bf), V((5, 4, S // 2, 128), bf),
               pltpu.SemaphoreType.DMA((32,)), pltpu.SemaphoreType.DMA((16,))])
        out = pl.pallas_call(kern, in_specs=[pl.BlockSpec(memory_space=pl.ANY)]*14, out_specs=pl.BlockSpec(memory_space=pl.ANY),
            out_shape=jax.ShapeDtypeStruct((S, 896), bf), scratch_shapes=scratch,
            compiler_params=pltpu.CompilerParams(vmem_limit_bytes=120<<20, flags=flags))(
            A_x.reshape(S, M).T, A_w_r.T, A_w_i.T, B_x.reshape(S, M).T, B_c_kv.reshape(S, DC), B_w_q.reshape(M*H, D),
            B_w_uk.reshape(DC*H, D), B_w_uv.reshape(DC*H, D), B_w_o.transpose(0, 2, 1), *consts)
        return out.reshape(1, S, 896)
    return fn


@jax.jit
def pallas_concat_heads__spectral_gfnet__compressed_kv_cla__prompt_kernel(
    A_x, A_w_r, A_w_i, B_x, B_c_kv, B_w_q, B_w_uk, B_w_uv, B_w_o,
):
    return make()(A_x, A_w_r, A_w_i, B_x, B_c_kv, B_w_q, B_w_uk, B_w_uv, B_w_o)
```

```python
import functools, math, contextlib
import numpy as np, jax, jax.numpy as jnp
import ml_dtypes
from jax import lax
from jax.experimental import pallas as pl
from jax.experimental.pallas import tpu as pltpu

S, M, H, D, DC = 2048, 448, 16, 256, 1024
DF = M // 2 + 1
HM = M // 2
f32, bf = jnp.float32, jnp.bfloat16
NT = (((1,), (1,)), ((), ()))
LOG2E = 1.4426950408889634
QSCALE = (D ** -0.5) * LOG2E
NEG = -1e9 * LOG2E

def _consts():
    nb = ml_dtypes.bfloat16
    d = np.arange(M, dtype=np.float64)
    f = np.arange(DF, dtype=np.float64)
    ang = 2 * np.pi * ((f[:, None] * d[None, :]) % M) / M
    cs, sn = np.cos(ang), np.sin(ang)
    HMc = M // 2
    FT = np.zeros((480, HMc))
    FT[0:113] = cs[0::2, :HMc]; FT[128:128 + 113] = -sn[0::2, :HMc]
    FT[256:256 + 112] = cs[1::2, :HMc]; FT[368:368 + 112] = -sn[1::2, :HMc]
    k1 = np.arange(16)[:, None, None]; k2 = np.arange(128)[None, :, None]; n2 = np.arange(128)[None, None, :]
    a = 2 * np.pi * ((n2 * (k1 + 16 * k2)) % S) / S
    Mr, Mi = np.cos(a), -np.sin(a)
    MF = np.concatenate([Mr, Mi], 2)
    MI = np.concatenate([np.transpose(Mr, (0, 2, 1)), -np.transpose(Mi, (0, 2, 1))], 2) / S
    c = np.full(DF, 2.0); c[0] = 1.0; c[-1] = 1.0
    Gc = (c[:, None] * cs) / M; Gs = -(c[:, None] * sn) / M
    G = np.zeros((2, HMc, 256))
    G[0, :, 0:113] = Gc[0::2, :HMc].T; G[0, :, 128:128 + 113] = Gs[0::2, :HMc].T
    G[1, :, 0:112] = Gc[1::2, :HMc].T; G[1, :, 128:128 + 112] = Gs[1::2, :HMc].T
    P = np.zeros((128, 128))
    for a_ in range(16):
        for j in range(8):
            P[a_ * 8 + j, 16 * j + a_] = 1.0
    return tuple(np.asarray(x, dtype=np.float32).astype(nb) for x in (FT, MF, MI, G, P))

_C = [math.cos(2 * math.pi * k / 16) for k in range(16)]
_S = [math.sin(2 * math.pi * k / 16) for k in range(16)]

def _cmul_tw(re, im, k, sign):
    k = k % 16
    c, s = _C[k], sign * _S[k]
    if k == 0: return re, im
    if k == 4: return (-sign * im, sign * re) if True else None
    if k == 8: return -re, -im
    if k == 12: return (sign * im, -sign * re)
    if k in (2, 6, 10, 14):
        h = math.sqrt(0.5)
        sc, ss = (1 if c > 0 else -1), (1 if s > 0 else -1)
        a = (re - im) if sc == ss else (re + im)
        b = (re + im) if sc == ss else (re - im)
        if sc == 1 and ss == 1: return (re - im) * h, (re + im) * h
        if sc == 1 and ss == -1: return (re + im) * h, (im - re) * h
        if sc == -1 and ss == 1: return (re + im) * (-h), (re - im) * h
        return (im - re) * h, (re + im) * (-h)
    return re * c - im * s, re * s + im * c

def _dft4(xs, sign):
    (a0, b0), (a1, b1), (a2, b2), (a3, b3) = xs
    sr, si = a0 + a2, b0 + b2
    dr, di = a0 - a2, b0 - b2
    tr, ti = a1 + a3, b1 + b3
    ur, ui = a1 - a3, b1 - b3
    if sign > 0:
        x1 = (dr - ui, di + ur); x3 = (dr + ui, di - ur)
    else:
        x1 = (dr + ui, di - ur); x3 = (dr - ui, di + ur)
    return [(sr + tr, si + ti), x1, (sr - tr, si - ti), x3]

def _fft16(xs, sign):
    t = [[None] * 4 for _ in range(4)]
    for b in range(4):
        y = _dft4([xs[4 * a + b] for a in range(4)], sign)
        for c in range(4):
            t[b][c] = _cmul_tw(y[c][0], y[c][1], b * c, sign)
    out = [None] * 16
    for c in range(4):
        y = _dft4([t[b][c] for b in range(4)], sign)
        for d in range(4):
            out[c + 4 * d] = y[d]
    return out

SCOPES = False
_cur = [None]
def mark(name):
    if not SCOPES: return
    if _cur[0] is not None:
        _cur[0].__exit__(None, None, None); _cur[0] = None
    if name is not None:
        _cur[0] = jax.named_scope(name); _cur[0].__enter__()

_SP = {1: ((11, 1), (22, 1)), 2: ((21, 1), (22, -1)), 3: ((12, 1), (22, 1)), 4: ((11, 1), (21, 1)),
       5: ((11, -1), (12, 1)), 6: ((22, 1),), 7: ((11, 1),)}
_CNT = {11: 4, 12: 2, 21: 2, 22: 4}

def make(order="S4", sbm=512, qbm=512, wmode=1, sorder=(1,2,3,4,5,6,7), bq=512, flags=None, oproj_bm=512, doA=True, doB=True, dft_unroll=4, wp_unroll=4, when=dict(c='qproj',wuk='qproj',wuv='qproj',wo='kvpre',g='kvpre'), pv_split=256):
    nq = S // bq
    sub = 128
    nsub = bq // sub
    XT = [(0, 128), (128, 128), (256, 128), (384, 64)]
    consts = _consts()

    def kern(ax_hbm, wr_hbm, wi_hbm, bx_hbm, c_hbm, wq_hbm, wuk_hbm, wuv_hbm, wo_hbm,
             ft_hbm, mf_hbm, mi_hbm, g_hbm, p_hbm, out_hbm,
             axT, wrT, wiT, ft, mf, mi, g, pm, rt, x1t, wp, y1, ys,
             x0, x1, c_s, wq_b, wuk_b, wuv_b,
             wq_s, wkv_s, q_all, k_s, v_s, out_s, xT, woT, pc, sems, osem):
        dmas = {}
        n = [0]
        def dma(name, src, dst):
            cp = pltpu.make_async_copy(src, dst, sems.at[n[0]])
            n[0] += 1
            dmas[name] = cp
        dma("ft", ft_hbm, ft)
        for t in range(4):
            dma(("ax", t), ax_hbm.at[:, pl.ds(512 * t, 512)], axT.at[:, pl.ds(512 * t, 512)])
        dma("pm", p_hbm, pm)
        dma("wr", wr_hbm, wrT)
        dma("wi", wi_hbm, wiT)
        for t in range(4):
            dma(("mf", t), mf_hbm.at[pl.ds(4 * t, 4)], mf.at[pl.ds(4 * t, 4)])
            dma(("mi", t), mi_hbm.at[pl.ds(4 * t, 4)], mi.at[pl.ds(4 * t, 4)])
            for hf in range(2):
                cols = pl.ds(hf * (S // 2) + 256 * t, 256)
                dma(("x", t, hf), bx_hbm.at[:, cols], xT.at[:, cols])
        for dt in range(2):
            dma(("wq", dt), wq_hbm.at[:, pl.ds(128 * dt, 128)], wq_b.at[dt])
        for t in range(8):
            dma(("c", t), c_hbm.at[:, pl.ds(128 * t, 128)], c_s.at[t])
        for dt in range(2):
            dma(("wuk", dt), wuk_hbm.at[:, pl.ds(128 * dt, 128)], wuk_b.at[dt])
        for dt in range(2):
            dma(("wuv", dt), wuv_hbm.at[:, pl.ds(128 * dt, 128)], wuv_b.at[dt])
        dma("g", g_hbm, g)
        dma("wo", wo_hbm, woT)
        started = set()
        def start(point):
            for name in dmas:
                key = name[0] if isinstance(name, tuple) else name
                if when.get(key, "begin") == point:
                    dmas[name].start(); started.add(name)
        start("begin")

        if doA:
            mark('A_zero')
            @pl.loop(0, 16)
            def _(k1):
                x1t[1, k1, 112:128, :] = jnp.zeros((16, 256), bf)
            @pl.loop(0, 16)
            def _(k1):
                for a in range(2):
                    for t in range(2):
                        wp[a, t, k1] = jnp.zeros((128, 128), f32)
            mark('A_dfwd'); start('A_dfwd')
            dmas["ft"].wait()
            for t in range(4):
                dmas[("ax", t)].wait()
                cols = slice(512 * t, 512 * (t + 1))
                lo = axT[0:HM, cols].astype(f32); hi = axT[HM:M, cols].astype(f32)
                rt[0:256, cols] = jnp.dot(ft[0:256, :], (lo + hi).astype(bf), preferred_element_type=f32)
                rt[256:480, cols] = jnp.dot(ft[256:480, :], (lo - hi).astype(bf), preferred_element_type=f32)
            mark('A_wperm'); start('A_wperm')
            def wperm(kt, cols, k2):
                for a, wref in enumerate((wrT, wiT)):
                    u = pltpu.bitcast(wref[0:HM, cols], jnp.int32)
                    ev = pltpu.bitcast(u << 16, f32).astype(bf)
                    od = pltpu.bitcast(u & jnp.int32(-65536), f32).astype(bf)
                    ev = jnp.concatenate([ev, wref[HM:DF, cols]], axis=0)
                    r0 = lax.dot_general(pm[...], ev, NT, preferred_element_type=f32)
                    r1 = lax.dot_general(pm[...], od, NT, preferred_element_type=f32)
                    for k1 in range(16):
                        wp[a, 0, k1, k2, 0:113] = r0[8 * k1:8 * k1 + 8]
                        wp[a, 1, k1, k2, 0:112] = r1[8 * k1:8 * k1 + 8]
            def fwd_fft(base_re, base_im, ftile, r0):
                halves = []
                for hf in range(2):
                    rr = pl.ds(base_re + r0 + 8 * hf, 8); ri = pl.ds(base_im + r0 + 8 * hf, 8)
                    zs = [(rt[rr, 128 * n1:128 * (n1 + 1)], rt[ri, 128 * n1:128 * (n1 + 1)]) for n1 in range(16)]
                    halves.append(_fft16(zs, -1))
                for k1 in range(16):
                    for p in range(2):
                        v = jnp.concatenate([halves[0][k1][p], halves[1][k1][p]], axis=0).astype(bf)
                        x1t[ftile, k1, pl.ds(r0, 16), 128 * p:128 * (p + 1)] = v
            if wmode == 0:
                @pl.loop(0, 8)
                def _(gi):
                    for u in range(2):
                        kt = gi * 2 + u
                        wperm(kt, pl.ds(pl.multiple_of(kt * 128, 128), 128), pl.ds(pl.multiple_of(kt * 8, 8), 8))
                    fwd_fft(0, 128, 0, pl.multiple_of(gi * 16, 16))
                    fwd_fft(256, 368, 1, pl.multiple_of(jnp.minimum(gi, 6) * 16, 16))
            elif wmode == 1:
                mark('A_ffft')
                lax.fori_loop(0, 8, lambda gi, _: fwd_fft(0, 128, 0, pl.multiple_of(gi * 16, 16)), None)
                lax.fori_loop(0, 7, lambda gi, _: fwd_fft(256, 368, 1, pl.multiple_of(gi * 16, 16)), None)
                mark('A_wperm')
                dmas["pm"].wait(); dmas["wr"].wait(); dmas["wi"].wait()
                for kt in range(16):
                    wperm(kt, slice(kt * 128, (kt + 1) * 128), slice(kt * 8, kt * 8 + 8))
            elif wmode == 2:
                @pl.loop(0, 8)
                def _(gi):
                    for u in range(2):
                        kt = gi * 2 + u
                        wperm(kt, pl.ds(pl.multiple_of(kt * 128, 128), 128), pl.ds(pl.multiple_of(kt * 8, 8), 8))
                    fwd_fft(0, 128, 0, pl.multiple_of(gi * 16, 16))
                lax.fori_loop(0, 7, lambda gi, _: fwd_fft(256, 368, 1, pl.multiple_of(gi * 16, 16)), None)
            elif wmode == 3:
                @pl.loop(0, 16)
                def _(kt):
                    wperm(kt, pl.ds(pl.multiple_of(kt * 128, 128), 128), pl.ds(pl.multiple_of(kt * 8, 8), 8))
                    t1 = kt >= 8
                    base_re = jnp.where(t1, 256, 0); base_im = jnp.where(t1, 368, 128)
                    g = jnp.minimum(kt, 14) % 8
                    fwd_fft(base_re, base_im, t1.astype(jnp.int32), pl.multiple_of(g * 16, 16))
            elif wmode == 4:
                lax.fori_loop(0, 7, lambda gi, _: fwd_fft(256, 368, 1, pl.multiple_of(gi * 16, 16)), None)
                @pl.loop(0, 4)
                def _(gi):
                    for u in range(4):
                        kt = gi * 4 + u
                        wperm(kt, pl.ds(pl.multiple_of(kt * 128, 128), 128), pl.ds(pl.multiple_of(kt * 8, 8), 8))
                    for u in range(2):
                        fwd_fft(0, 128, 0, pl.multiple_of((gi * 2 + u) * 16, 16))
            mark('A_dft128'); start('A_dft128')
            def realform(m):
                r_, i_ = m[:, :128], m[:, 128:]
                ni = pltpu.bitcast(pltpu.bitcast(i_, jnp.int32) ^ jnp.int32(-2147450880), bf)
                return jnp.concatenate([jnp.concatenate([r_, ni], axis=1), jnp.concatenate([i_, r_], axis=1)], axis=0)
            def d1(k1):
                xt = jnp.concatenate([x1t[0, k1], x1t[1, k1]], axis=0)
                return lax.dot_general(realform(mf[k1]), xt, NT, preferred_element_type=f32)
            def d2(k1, x2):
                xr, xi = x2[:128], x2[128:]
                wr_ = jnp.concatenate([wp[0, 0, k1], wp[0, 1, k1]], axis=1)
                wi_ = jnp.concatenate([wp[1, 0, k1], wp[1, 1, k1]], axis=1)
                z = jnp.concatenate([xr * wr_ - xi * wi_, xr * wi_ + xi * wr_], axis=0).astype(bf)
                y = jnp.dot(realform(mi[k1]), z, preferred_element_type=f32)
                y1[0, k1] = y[:, :128]
                y1[1, k1] = y[:, 128:]
            if dft_unroll == 16:
                for kb in range(4):
                    dmas[("mf", kb)].wait(); dmas[("mi", kb)].wait()
                    x2s = [d1(kb * 4 + u) for u in range(4)]
                    for u in range(4):
                        d2(kb * 4 + u, x2s[u])
                    for t, (o, w) in enumerate(XT):
                        for sb in range(4):
                            rr = slice(kb * 512 + sb * 128, kb * 512 + (sb + 1) * 128)
                            xs[t][rr, :] = xT[o:o+w, rr].T
            else:
                sem_mf = list(dmas).index(("mf", 0))
                @pl.loop(0, 4)
                def _(kb):
                    blk = pl.ds(4 * kb, 4)
                    pltpu.make_async_copy(mf_hbm.at[blk], mf.at[blk], sems.at[sem_mf + 4 * kb]).wait()
                    pltpu.make_async_copy(mi_hbm.at[blk], mi.at[blk], sems.at[sem_mf + 4 * kb + 1]).wait()
                    for hf in range(2):
                        cols = pl.ds(pl.multiple_of(hf * (S // 2) + 256 * kb, 256), 256)
                        pltpu.make_async_copy(bx_hbm.at[:, cols], xT.at[:, cols], sems.at[sem_mf + 4 * kb + 2 + hf]).wait()
                    x2s = [d1(kb * 4 + u) for u in range(4)]
                    for u in range(4):
                        d2(kb * 4 + u, x2s[u])
                    for sb in range(2):
                        c0 = pl.multiple_of(kb * 256 + sb * 128, 128)
                        lo = pl.ds(c0, 128); hi = pl.ds(S // 2 + c0, 128)
                        a11 = xT[0:HM, lo].astype(f32); a12 = xT[HM:M, lo].astype(f32)
                        a21 = xT[0:HM, hi].astype(f32); a22 = xT[HM:M, hi].astype(f32)
                        for i, pv_ in enumerate((a11 + a22, a21 + a22, a11, a22, a11 + a12, a21 - a11, a12 - a22)):
                            x0[i, lo, :] = pv_[0:128].T.astype(bf)
                            x1[i, lo, :] = pv_[128:HM].T.astype(bf)

        mark('qproj'); start('qproj')
        dmas[("wq", 0)].wait()
        wq_i = wq_b.bitcast(jnp.int32)
        def inv_fft(r0):
            for t in range(2):
                halves = []
                for hf in range(2):
                    rr = pl.ds(r0 + 8 * hf, 8); ri = pl.ds(128 + r0 + 8 * hf, 8)
                    zs = [(y1[t, k1, rr, :], y1[t, k1, ri, :]) for k1 in range(16)]
                    halves.append(_fft16(zs, 1))
                for n1 in range(16):
                    for p in range(2):
                        v = jnp.concatenate([halves[0][n1][p], halves[1][n1][p]], axis=0).astype(bf)
                        ys[2 * p + t, pl.ds(128 * n1 + r0, 16), :] = v
        def extract_q(it):
            dt = it // 4
            for pb in range(2):
                p = 2 * (it % 4) + pb
                u = wq_i.at[dt, pl.ds(p, M * 8 - 7)][pl.ds(0, M, stride=8), :]
                lo = pltpu.bitcast(u << 16, f32)
                hi = pltpu.bitcast(u & jnp.int32(-65536), f32)
                b11, b12, b21, b22 = lo[:HM], hi[:HM], lo[HM:], hi[HM:]
                for i, qv in enumerate((b11 + b22, b11, b12 - b22, b21 - b11, b22, b11 + b12, b21 + b22)):
                    wq_s[i, pb] = qv.astype(bf)
        extract_q(0)
        def qbody(it, _):
            @pl.when(it == 3)
            def _():
                dmas[("wq", 1)].wait()
            dt = it // 4
            h0 = 4 * (it % 4)
            st = {}
            for ch in range(S // 2 // qbm):
                for i in sorder:
                    rows = slice(ch * qbm, (ch + 1) * qbm)
                    lhs = jnp.concatenate([x0[i - 1, rows, :], x1[i - 1, rows, :]], axis=1)
                    w = jnp.concatenate([wq_s[i - 1, 0], wq_s[i - 1, 1]], axis=1)
                    m = jnp.dot(lhs, w, preferred_element_type=f32)
                    for blk, sign in _SP[i]:
                        key = (blk, ch)
                        if key not in st:
                            st[key] = [m if sign > 0 else -m, 1]
                        else:
                            st[key][0] = st[key][0] + m if sign > 0 else st[key][0] - m
                            st[key][1] += 1
                        if st[key][1] == _CNT[blk]:
                            r = (st.pop(key)[0] * QSCALE).astype(bf)
                            base = (blk // 10 - 1) * (S // 2) + ch * qbm
                            hh = h0 + (blk % 10 - 1)
                            q_all[2 * hh + dt, base:base + qbm, :] = r[:, :128]
                            q_all[2 * (hh + 2) + dt, base:base + qbm, :] = r[:, 128:]
            extract_q(jnp.minimum(it + 1, 7))
            inv_fft(pl.multiple_of(it * 16, 16))
        lax.fori_loop(0, 8, qbody, None)

        mark('kvpre'); start('kvpre')
        for t in range(8): dmas[("c", t)].wait()
        for dt in range(2): dmas[("wuk", dt)].wait(); dmas[("wuv", dt)].wait()
        wuk_i = wuk_b.bitcast(jnp.int32)
        wuv_i = wuv_b.bitcast(jnp.int32)
        HK = DC // 2
        def extract_kv(h):
            j = h // 2
            sh = (1 - h % 2) * 16
            for a, wi in enumerate((wuk_i, wuv_i)):
                b = {}
                for dt in range(2):
                    u = wi.at[dt, pl.ds(j, DC * 8 - 7)][pl.ds(0, DC, stride=8), :]
                    w = pltpu.bitcast((u << sh) & jnp.int32(-65536), f32)
                    b[(0, dt)] = w[:HK]; b[(1, dt)] = w[HK:]
                b11, b12, b21, b22 = b[(0, 0)], b[(0, 1)], b[(1, 0)], b[(1, 1)]
                for i, qv in enumerate((b11 + b22, b11, b12 - b22, b21 - b11, b22, b11 + b12, b21 + b22)):
                    wkv_s[i, a] = qv.astype(bf)
        extract_kv(0)
        HS = S // 2
        @pl.loop(0, HS // 128)
        def _(gi):
            r0 = pl.multiple_of(gi * 128, 128)
            top = pl.ds(r0, 128); bot = pl.ds(HS + r0, 128)
            for t in range(4):
                a11 = c_s[t, top, :].astype(f32); a12 = c_s[4 + t, top, :].astype(f32)
                a21 = c_s[t, bot, :].astype(f32); a22 = c_s[4 + t, bot, :].astype(f32)
                for i, pv_ in enumerate((a11 + a22, a21 + a22, a11 + a12, a21 - a11, a12 - a22)):
                    pc[i, t, top, :] = pv_.astype(bf)

        row = lax.broadcasted_iota(jnp.int32, (sub, sub), 0)
        col = lax.broadcasted_iota(jnp.int32, (sub, sub), 1)
        tri = col <= row

        def hbody(h, _):
            st = {}
            def qload(r0, r1):
                return jnp.concatenate([q_all[2 * h, r0:r1, :], q_all[2 * h + 1, r0:r1, :]], axis=1)
            def kload(r0, r1):
                return jnp.concatenate([k_s[0, r0:r1, :], k_s[1, r0:r1, :]], axis=1)
            def vload(r0, r1):
                return jnp.concatenate([v_s[0, r0:r1, :], v_s[1, r0:r1, :]], axis=1)
            def sp(i, ch):
                rows = slice(ch * sbm, (ch + 1) * sbm)
                if i == 3:
                    lhs = [c_s[t, rows, :] for t in range(4)]
                elif i == 4:
                    lhs = [c_s[4 + t, HS + ch * sbm:HS + (ch + 1) * sbm, :] for t in range(4)]
                else:
                    pi = {1: 0, 2: 1, 5: 2, 6: 3, 7: 4}[i]
                    lhs = [pc[pi, t, rows, :] for t in range(4)]
                w = jnp.concatenate([wkv_s[i - 1, 0], wkv_s[i - 1, 1]], axis=1)
                m = jnp.dot(jnp.concatenate(lhs, axis=1), w, preferred_element_type=f32)
                for blk, sign in {1: ((11, 1), (22, 1)), 2: ((21, 1), (22, -1)), 3: ((12, 1), (22, 1)), 4: ((11, 1), (21, 1)),
                                  5: ((11, -1), (12, 1)), 6: ((22, 1),), 7: ((11, 1),)}[i]:
                    key = ("c", blk, ch)
                    if key not in st:
                        st[key] = [m if sign > 0 else -m, 1]
                    else:
                        st[key][0] = st[key][0] + m if sign > 0 else st[key][0] - m
                        st[key][1] += 1
                    if st[key][1] == {11: 4, 12: 2, 21: 2, 22: 4}[blk]:
                        r = st.pop(key)[0].astype(bf)
                        base = (blk // 10 - 1) * HS + ch * sbm
                        dt = blk % 10 - 1
                        k_s[dt, base:base + sbm, :] = r[:, :128]
                        v_s[dt, base:base + sbm, :] = r[:, 128:]
            def qk(i, j):
                if j < i:
                    s = lax.dot_general(qload(i*bq, (i+1)*bq), kload(j*bq, (j+1)*bq), NT, preferred_element_type=f32)
                    st[("s", i, j)] = s
                    mj = jnp.max(s, axis=1, keepdims=True)
                else:
                    parts = [[] for _ in range(nsub)]
                    for t in range(nsub):
                        r0 = t * sub
                        s = lax.dot_general(qload(i*bq + r0, (i+1)*bq), kload(j*bq + r0, j*bq + r0 + sub), NT, preferred_element_type=f32)
                        parts[t].append(jnp.where(tri, s[:sub], NEG))
                        for r in range(t + 1, nsub):
                            parts[r].append(s[(r-t)*sub:(r-t+1)*sub])
                    st[("sd", i)] = parts
                    ms = [jnp.max(functools.reduce(jnp.maximum, parts[r]), axis=1, keepdims=True) for r in range(nsub)]
                    mj = jnp.concatenate(ms, axis=0)
                st[("m", i)] = mj if ("m", i) not in st else jnp.maximum(st[("m", i)], mj)
            def pv(i, j):
                m = st[("m", i)]
                if j < i:
                    sfull = st.pop(("s", i, j))
                    for c0 in range(0, bq, pv_split):
                        p = jnp.exp2(sfull[:, c0:c0 + pv_split] - m)
                        lj = functools.reduce(jnp.add, [p[:, t*sub:(t+1)*sub] for t in range(pv_split // sub)])
                        o = jnp.dot(p.astype(bf), vload(j*bq + c0, j*bq + c0 + pv_split), preferred_element_type=f32)
                        st[("l", i)] = lj if ("l", i) not in st else st[("l", i)] + lj
                        st[("o", i)] = o if ("o", i) not in st else st[("o", i)] + o
                else:
                    parts = st.pop(("sd", i))
                    for r in range(nsub):
                        rows = slice(r*sub, (r+1)*sub)
                        w = (r+1)*sub
                        ps = [jnp.exp2(x - m[rows]) for x in parts[r]]
                        lj = functools.reduce(jnp.add, ps)
                        p = jnp.concatenate(ps, axis=1) if r > 0 else ps[0]
                        o = jnp.dot(p.astype(bf), vload(j*bq, j*bq + w), preferred_element_type=f32)
                        if ("l", i) in st:
                            lj = lj + st[("l", i)][rows]; o = o + st[("o", i)][rows]
                        l = jnp.sum(lj, axis=1, keepdims=True)
                        rl = pl.reciprocal(l, approx=True)
                        rl = rl * (2.0 - l * rl)
                        ctx = (o * rl).astype(bf)
                        rr = slice(i*bq + r*sub, i*bq + (r+1)*sub)
                        q_all[2 * h, rr, :] = ctx[:, :128]
                        q_all[2 * h + 1, rr, :] = ctx[:, 128:]
            att = []
            for i in range(nq - 2, -2, -1):
                a = [("qk", i, j) for j in range(i+1)] if i >= 0 else []
                b = [("pv", i+1, j) for j in range(i+2)]
                for t in range(max(len(a), len(b))):
                    if t < len(a): att.append(a[t])
                    if t < len(b): att.append(b[t])
            P = sorder
            if order == "S1":
                seq = [("sp", i, 0) for i in P] + [("qk", 3, 0)] + [("sp", i, 1) for i in P[:3]] + [("qk", 3, 2)] + [("sp", i, 1) for i in P[3:]] + [("qk", 3, 1), ("qk", 3, 3), ("ex",)] + att
            elif order == "S2":
                seq = [("sp", i, 0) for i in P] + [("sp", i, 1) for i in P] + [("qk", 3, j) for j in range(4)] + [("ex",)] + att
            elif order == "S3":
                seq = [("sp", i, 0) for i in P] + [("sp", i, 1) for i in P] + [("ex",)] + [("qk", 3, j) for j in range(4)] + att
            elif order == "S4":
                seq = [("sp", i, 0) for i in P] + [("qk", 3, 0), ("qk", 3, 2)] + [("sp", i, 1) for i in P] + [("qk", 3, 1), ("qk", 3, 3), ("ex",)] + att
            else:
                seq = order
            if sbm == 1024:
                seq = [("sp", i, 0) for i in P] + [("qk", 3, j) for j in range(4)] + [("ex",)] + att
            for op in seq:
                if op[0] == "sp": sp(*op[1:])
                elif op[0] == "qk": qk(*op[1:])
                elif op[0] == "pv": pv(*op[1:])
                elif op[0] == "ex": extract_kv(jnp.minimum(h + 1, H - 1))
        lax.fori_loop(0, H, hbody, None)

        mark('oproj'); start('oproj')
        dmas["wo"].wait(); dmas["g"].wait()
        nt_per = oproj_bm // 128
        def obody(m, _):
            for u in range(nt_per):
                r0 = pl.multiple_of(m * oproj_bm + u * 128, 128)
                rows = pl.ds(r0, 128)
                ye = jnp.concatenate([ys[0, rows, :], ys[2, rows, :]], axis=1)
                yo = jnp.concatenate([ys[1, rows, :], ys[3, rows, :]], axis=1)
                ev = lax.dot_general(g[0], ye, NT, preferred_element_type=f32)
                od = lax.dot_general(g[1], yo, NT, preferred_element_type=f32)
                at = jnp.concatenate([ev + od, ev - od], axis=0)
                ctx = jnp.concatenate([q_all[t, rows, :] for t in range(32)], axis=1)
                w = jnp.concatenate([woT[hh] for hh in range(H)], axis=1)
                bt = lax.dot_general(w, ctx, NT, preferred_element_type=f32)
                tt = jnp.concatenate([at, bt], axis=0)
                for c in range(7):
                    out_s[rows, c * 128:(c + 1) * 128] = tt[c * 128:(c + 1) * 128].T.astype(bf)
                pltpu.make_async_copy(out_s.at[rows], out_hbm.at[rows], osem.at[m * nt_per + u]).start()
        lax.fori_loop(0, S // oproj_bm, obody, None)
        mark('owait')
        def owait(m, _):
            rows = pl.ds(pl.multiple_of(m * 128, 128), 128)
            pltpu.make_async_copy(out_s.at[rows], out_hbm.at[rows], osem.at[m]).wait()
        lax.fori_loop(0, S // 128, owait, None)
        mark(None)

    def fn(A_x, A_w_r, A_w_i, B_x, B_c_kv, B_w_q, B_w_uk, B_w_uv, B_w_o):
        V = pltpu.VMEM
        scratch = ([V((M, S), bf), V((DF, S), bf), V((DF, S), bf), V((480, HM), bf), V((16, 128, 256), bf), V((16, 128, 256), bf),
                    V((2, HM, 256), bf), V((128, 128), bf), V((480, S), f32), V((2, 16, 128, 256), bf), V((2, 2, 16, 128, 128), f32),
                    V((2, 16, 256, 128), f32), V((4, S, 128), bf)]
            + [V((7, S // 2, 128), bf), V((7, S // 2, HM - 128), bf)] + [V((8, S, 128), bf), V((2, M*H, 128), bf), V((2, DC*H, 128), bf), V((2, DC*H, 128), bf)]
            + [V((7, 2, HM, 128), bf), V((7, 2, DC // 2, 128), bf), V((32, S, 128), bf), V((2, S, 128), bf), V((2, S, 128), bf), V((S, 896), bf),
               V((M, S), bf), V((H, M, D), bf), V((5, 4, S // 2, 128), bf),
               pltpu.SemaphoreType.DMA((48,)), pltpu.SemaphoreType.DMA((16,))])
        out = pl.pallas_call(kern, in_specs=[pl.BlockSpec(memory_space=pl.ANY)]*14, out_specs=pl.BlockSpec(memory_space=pl.ANY),
            out_shape=jax.ShapeDtypeStruct((S, 896), bf), scratch_shapes=scratch,
            compiler_params=pltpu.CompilerParams(vmem_limit_bytes=120<<20, flags=flags))(
            A_x.reshape(S, M).T, A_w_r.T, A_w_i.T, B_x.reshape(S, M).T, B_c_kv.reshape(S, DC), B_w_q.reshape(M*H, D),
            B_w_uk.reshape(DC*H, D), B_w_uv.reshape(DC*H, D), B_w_o.transpose(0, 2, 1), *consts)
        return out.reshape(1, S, 896)
    return fn


@jax.jit
def pallas_concat_heads__spectral_gfnet__compressed_kv_cla__prompt_kernel(
    A_x, A_w_r, A_w_i, B_x, B_c_kv, B_w_q, B_w_uk, B_w_uv, B_w_o,
):
    return make()(A_x, A_w_r, A_w_i, B_x, B_c_kv, B_w_q, B_w_uk, B_w_uv, B_w_o)
```

```python
import functools, math
import numpy as np, jax, jax.numpy as jnp
import ml_dtypes
from jax import lax
from jax.experimental import pallas as pl
from jax.experimental.pallas import tpu as pltpu

S, M, H, D, DC = 2048, 448, 16, 256, 1024
DF = M // 2 + 1
HM = M // 2
f32, bf = jnp.float32, jnp.bfloat16
NT = (((1,), (1,)), ((), ()))
LOG2E = 1.4426950408889634
QSCALE = (D ** -0.5) * LOG2E
NEG = -1e9 * LOG2E

def _consts():
    nb = ml_dtypes.bfloat16
    d = np.arange(M, dtype=np.float64)
    f = np.arange(DF, dtype=np.float64)
    ang = 2 * np.pi * ((f[:, None] * d[None, :]) % M) / M
    cs, sn = np.cos(ang), np.sin(ang)
    HMc = M // 2
    FT = np.zeros((480, HMc))
    FT[0:113] = cs[0::2, :HMc]; FT[128:128 + 113] = -sn[0::2, :HMc]
    FT[256:256 + 112] = cs[1::2, :HMc]; FT[368:368 + 112] = -sn[1::2, :HMc]
    k1 = np.arange(16)[:, None, None]; k2 = np.arange(128)[None, :, None]; n2 = np.arange(128)[None, None, :]
    a = 2 * np.pi * ((n2 * (k1 + 16 * k2)) % S) / S
    Mr, Mi = np.cos(a), -np.sin(a)
    MF = np.concatenate([Mr, Mi], 2)
    MI = np.concatenate([np.transpose(Mr, (0, 2, 1)), -np.transpose(Mi, (0, 2, 1))], 2) / S
    c = np.full(DF, 2.0); c[0] = 1.0; c[-1] = 1.0
    Gc = (c[:, None] * cs) / M; Gs = -(c[:, None] * sn) / M
    G = np.zeros((2, HMc, 256))
    G[0, :, 0:113] = Gc[0::2, :HMc].T; G[0, :, 128:128 + 113] = Gs[0::2, :HMc].T
    G[1, :, 0:112] = Gc[1::2, :HMc].T; G[1, :, 128:128 + 112] = Gs[1::2, :HMc].T
    P = np.zeros((128, 128))
    for a_ in range(16):
        for j in range(8):
            P[a_ * 8 + j, 16 * j + a_] = 1.0
    return tuple(np.asarray(x, dtype=np.float32).astype(nb) for x in (FT, MF, MI, G, P))

_C = [math.cos(2 * math.pi * k / 16) for k in range(16)]
_S = [math.sin(2 * math.pi * k / 16) for k in range(16)]

def _cmul_tw(re, im, k, sign):
    k = k % 16
    c, s = _C[k], sign * _S[k]
    if k == 0: return re, im
    if k == 4: return (-sign * im, sign * re) if True else None
    if k == 8: return -re, -im
    if k == 12: return (sign * im, -sign * re)
    if k in (2, 6, 10, 14):
        h = math.sqrt(0.5)
        sc, ss = (1 if c > 0 else -1), (1 if s > 0 else -1)
        a = (re - im) if sc == ss else (re + im)
        b = (re + im) if sc == ss else (re - im)
        if sc == 1 and ss == 1: return (re - im) * h, (re + im) * h
        if sc == 1 and ss == -1: return (re + im) * h, (im - re) * h
        if sc == -1 and ss == 1: return (re + im) * (-h), (re - im) * h
        return (im - re) * h, (re + im) * (-h)
    return re * c - im * s, re * s + im * c

def _dft4(xs, sign):
    (a0, b0), (a1, b1), (a2, b2), (a3, b3) = xs
    sr, si = a0 + a2, b0 + b2
    dr, di = a0 - a2, b0 - b2
    tr, ti = a1 + a3, b1 + b3
    ur, ui = a1 - a3, b1 - b3
    if sign > 0:
        x1 = (dr - ui, di + ur); x3 = (dr + ui, di - ur)
    else:
        x1 = (dr + ui, di - ur); x3 = (dr - ui, di + ur)
    return [(sr + tr, si + ti), x1, (sr - tr, si - ti), x3]

def _fft16(xs, sign):
    t = [[None] * 4 for _ in range(4)]
    for b in range(4):
        y = _dft4([xs[4 * a + b] for a in range(4)], sign)
        for c in range(4):
            t[b][c] = _cmul_tw(y[c][0], y[c][1], b * c, sign)
    out = [None] * 16
    for c in range(4):
        y = _dft4([t[b][c] for b in range(4)], sign)
        for d in range(4):
            out[c + 4 * d] = y[d]
    return out

_SP = {1: ((11, 1), (22, 1)), 2: ((21, 1), (22, -1)), 3: ((12, 1), (22, 1)), 4: ((11, 1), (21, 1)),
       5: ((11, -1), (12, 1)), 6: ((22, 1),), 7: ((11, 1),)}
_CNT = {11: 4, 12: 2, 21: 2, 22: 4}

def make(bq=512, sbm=512, qbm=512, oproj_bm=512, pv_split=256, flags=None, sorder=(1, 4, 5, 7, 2, 3, 6),
         when=dict(c='qproj', wuk='qproj', wuv='qproj', wo='kvpre', g='kvpre'), doA=True):
    nq = S // bq
    sub = 128
    nsub = bq // sub
    XT = [(0, 128), (128, 128), (256, 128), (384, 64)]
    consts = _consts()

    def kern(ax_hbm, wr_hbm, wi_hbm, bx_hbm, c_hbm, wq_hbm, wuk_hbm, wuv_hbm, wo_hbm,
             ft_hbm, mf_hbm, mi_hbm, g_hbm, p_hbm, out_hbm,
             axT, wrT, wiT, ft, mf, mi, g, pm, rt, x1t, wp, y1, ys,
             x0, x1, c_s, wq_b, wuk_b, wuv_b,
             wq_s, wkv_s, q_all, k_s, v_s, out_s, xT, woT, pc, sems, osem):
        dmas = {}
        n = [0]
        def dma(name, src, dst):
            cp = pltpu.make_async_copy(src, dst, sems.at[n[0]])
            n[0] += 1
            dmas[name] = cp
        dma("ft", ft_hbm, ft)
        for t in range(4):
            dma(("ax", t), ax_hbm.at[:, pl.ds(512 * t, 512)], axT.at[:, pl.ds(512 * t, 512)])
        dma("pm", p_hbm, pm)
        dma("wr", wr_hbm, wrT)
        dma("wi", wi_hbm, wiT)
        for t in range(4):
            dma(("mf", t), mf_hbm.at[pl.ds(4 * t, 4)], mf.at[pl.ds(4 * t, 4)])
            dma(("mi", t), mi_hbm.at[pl.ds(4 * t, 4)], mi.at[pl.ds(4 * t, 4)])
            for hf in range(2):
                cols = pl.ds(hf * (S // 2) + 256 * t, 256)
                dma(("x", t, hf), bx_hbm.at[:, cols], xT.at[:, cols])
        for dt in range(2):
            dma(("wq", dt), wq_hbm.at[:, pl.ds(128 * dt, 128)], wq_b.at[dt])
        for t in range(8):
            dma(("c", t), c_hbm.at[:, pl.ds(128 * t, 128)], c_s.at[t])
        for dt in range(2):
            dma(("wuk", dt), wuk_hbm.at[:, pl.ds(128 * dt, 128)], wuk_b.at[dt])
        for dt in range(2):
            dma(("wuv", dt), wuv_hbm.at[:, pl.ds(128 * dt, 128)], wuv_b.at[dt])
        dma("g", g_hbm, g)
        dma("wo", wo_hbm, woT)
        started = set()
        def start(point):
            for name in dmas:
                key = name[0] if isinstance(name, tuple) else name
                if when.get(key, "begin") == point:
                    dmas[name].start(); started.add(name)
        start("begin")

        if doA:
            @pl.loop(0, 16)
            def _(k1):
                x1t[1, k1, 112:128, :] = jnp.zeros((16, 256), bf)
            @pl.loop(0, 16)
            def _(k1):
                for a in range(2):
                    for t in range(2):
                        wp[a, t, k1] = jnp.zeros((128, 128), f32)
            start('A_dfwd')
            dmas["ft"].wait()
            for t in range(4):
                dmas[("ax", t)].wait()
                cols = slice(512 * t, 512 * (t + 1))
                lo = axT[0:HM, cols].astype(f32); hi = axT[HM:M, cols].astype(f32)
                rt[0:256, cols] = jnp.dot(ft[0:256, :], (lo + hi).astype(bf), preferred_element_type=f32)
                rt[256:480, cols] = jnp.dot(ft[256:480, :], (lo - hi).astype(bf), preferred_element_type=f32)
            start('A_wperm')
            def wperm(kt, cols, k2):
                for a, wref in enumerate((wrT, wiT)):
                    u = pltpu.bitcast(wref[0:HM, cols], jnp.int32)
                    ev = pltpu.bitcast(u << 16, f32).astype(bf)
                    od = pltpu.bitcast(u & jnp.int32(-65536), f32).astype(bf)
                    ev = jnp.concatenate([ev, wref[HM:DF, cols]], axis=0)
                    r0 = lax.dot_general(pm[...], ev, NT, preferred_element_type=f32)
                    r1 = lax.dot_general(pm[...], od, NT, preferred_element_type=f32)
                    for k1 in range(16):
                        wp[a, 0, k1, k2, 0:113] = r0[8 * k1:8 * k1 + 8]
                        wp[a, 1, k1, k2, 0:112] = r1[8 * k1:8 * k1 + 8]
            def fwd_fft(base_re, base_im, ftile, r0):
                halves = []
                for hf in range(2):
                    rr = pl.ds(base_re + r0 + 8 * hf, 8); ri = pl.ds(base_im + r0 + 8 * hf, 8)
                    zs = [(rt[rr, 128 * n1:128 * (n1 + 1)], rt[ri, 128 * n1:128 * (n1 + 1)]) for n1 in range(16)]
                    halves.append(_fft16(zs, -1))
                for k1 in range(16):
                    for p in range(2):
                        v = jnp.concatenate([halves[0][k1][p], halves[1][k1][p]], axis=0).astype(bf)
                        x1t[ftile, k1, pl.ds(r0, 16), 128 * p:128 * (p + 1)] = v
            lax.fori_loop(0, 8, lambda gi, _: fwd_fft(0, 128, 0, pl.multiple_of(gi * 16, 16)), None)
            lax.fori_loop(0, 7, lambda gi, _: fwd_fft(256, 368, 1, pl.multiple_of(gi * 16, 16)), None)
            dmas["pm"].wait(); dmas["wr"].wait(); dmas["wi"].wait()
            for kt in range(16):
                wperm(kt, slice(kt * 128, (kt + 1) * 128), slice(kt * 8, kt * 8 + 8))
            start('A_dft128')
            def realform(m):
                r_, i_ = m[:, :128], m[:, 128:]
                ni = pltpu.bitcast(pltpu.bitcast(i_, jnp.int32) ^ jnp.int32(-2147450880), bf)
                return jnp.concatenate([jnp.concatenate([r_, ni], axis=1), jnp.concatenate([i_, r_], axis=1)], axis=0)
            def d1(k1):
                xt = jnp.concatenate([x1t[0, k1], x1t[1, k1]], axis=0)
                return lax.dot_general(realform(mf[k1]), xt, NT, preferred_element_type=f32)
            def d2(k1, x2):
                xr, xi = x2[:128], x2[128:]
                wr_ = jnp.concatenate([wp[0, 0, k1], wp[0, 1, k1]], axis=1)
                wi_ = jnp.concatenate([wp[1, 0, k1], wp[1, 1, k1]], axis=1)
                z = jnp.concatenate([xr * wr_ - xi * wi_, xr * wi_ + xi * wr_], axis=0).astype(bf)
                y = jnp.dot(realform(mi[k1]), z, preferred_element_type=f32)
                y1[0, k1] = y[:, :128]
                y1[1, k1] = y[:, 128:]
            sem_mf = list(dmas).index(("mf", 0))
            @pl.loop(0, 4)
            def _(kb):
                blk = pl.ds(4 * kb, 4)
                pltpu.make_async_copy(mf_hbm.at[blk], mf.at[blk], sems.at[sem_mf + 4 * kb]).wait()
                pltpu.make_async_copy(mi_hbm.at[blk], mi.at[blk], sems.at[sem_mf + 4 * kb + 1]).wait()
                for hf in range(2):
                    cols = pl.ds(pl.multiple_of(hf * (S // 2) + 256 * kb, 256), 256)
                    pltpu.make_async_copy(bx_hbm.at[:, cols], xT.at[:, cols], sems.at[sem_mf + 4 * kb + 2 + hf]).wait()
                x2s = [d1(kb * 4 + u) for u in range(4)]
                for u in range(4):
                    d2(kb * 4 + u, x2s[u])
                for sb in range(2):
                    c0 = pl.multiple_of(kb * 256 + sb * 128, 128)
                    lo = pl.ds(c0, 128); hi = pl.ds(S // 2 + c0, 128)
                    a11 = xT[0:HM, lo].astype(f32); a12 = xT[HM:M, lo].astype(f32)
                    a21 = xT[0:HM, hi].astype(f32); a22 = xT[HM:M, hi].astype(f32)
                    for i, pv_ in enumerate((a11 + a22, a21 + a22, a11, a22, a11 + a12, a21 - a11, a12 - a22)):
                        x0[i, lo, :] = pv_[0:128].T.astype(bf)
                        x1[i, lo, :] = pv_[128:HM].T.astype(bf)

        start('qproj')
        dmas[("wq", 0)].wait()
        wq_i = wq_b.bitcast(jnp.int32)
        def inv_fft(r0):
            for t in range(2):
                halves = []
                for hf in range(2):
                    rr = pl.ds(r0 + 8 * hf, 8); ri = pl.ds(128 + r0 + 8 * hf, 8)
                    zs = [(y1[t, k1, rr, :], y1[t, k1, ri, :]) for k1 in range(16)]
                    halves.append(_fft16(zs, 1))
                for n1 in range(16):
                    for p in range(2):
                        v = jnp.concatenate([halves[0][n1][p], halves[1][n1][p]], axis=0).astype(bf)
                        ys[2 * p + t, pl.ds(128 * n1 + r0, 16), :] = v
        def extract_q(it):
            dt = it // 4
            for pb in range(2):
                p = 2 * (it % 4) + pb
                u = wq_i.at[dt, pl.ds(p, M * 8 - 7)][pl.ds(0, M, stride=8), :]
                lo = pltpu.bitcast(u << 16, f32)
                hi = pltpu.bitcast(u & jnp.int32(-65536), f32)
                b11, b12, b21, b22 = lo[:HM], hi[:HM], lo[HM:], hi[HM:]
                for i, qv in enumerate((b11 + b22, b11, b12 - b22, b21 - b11, b22, b11 + b12, b21 + b22)):
                    wq_s[i, pb] = qv.astype(bf)
        extract_q(0)
        def qbody(it, _):
            @pl.when(it == 3)
            def _w():
                dmas[("wq", 1)].wait()
            dt = it // 4
            h0 = 4 * (it % 4)
            st = {}
            for ch in range(S // 2 // qbm):
                for i in sorder:
                    rows = slice(ch * qbm, (ch + 1) * qbm)
                    lhs = jnp.concatenate([x0[i - 1, rows, :], x1[i - 1, rows, :]], axis=1)
                    w = jnp.concatenate([wq_s[i - 1, 0], wq_s[i - 1, 1]], axis=1)
                    m = jnp.dot(lhs, w, preferred_element_type=f32)
                    for blk, sign in _SP[i]:
                        key = (blk, ch)
                        if key not in st:
                            st[key] = [m if sign > 0 else -m, 1]
                        else:
                            st[key][0] = st[key][0] + m if sign > 0 else st[key][0] - m
                            st[key][1] += 1
                        if st[key][1] == _CNT[blk]:
                            r = (st.pop(key)[0] * QSCALE).astype(bf)
                            base = (blk // 10 - 1) * (S // 2) + ch * qbm
                            hh = h0 + (blk % 10 - 1)
                            q_all[2 * hh + dt, base:base + qbm, :] = r[:, :128]
                            q_all[2 * (hh + 2) + dt, base:base + qbm, :] = r[:, 128:]
            extract_q(jnp.minimum(it + 1, 7))
            inv_fft(pl.multiple_of(it * 16, 16))
        lax.fori_loop(0, 8, qbody, None)

        start('kvpre')
        for t in range(8): dmas[("c", t)].wait()
        for dt in range(2): dmas[("wuk", dt)].wait(); dmas[("wuv", dt)].wait()
        wuk_i = wuk_b.bitcast(jnp.int32)
        wuv_i = wuv_b.bitcast(jnp.int32)
        HK = DC // 2
        def extract_kv(h):
            j = h // 2
            sh = (1 - h % 2) * 16
            for a, wi in enumerate((wuk_i, wuv_i)):
                b = {}
                for dt in range(2):
                    u = wi.at[dt, pl.ds(j, DC * 8 - 7)][pl.ds(0, DC, stride=8), :]
                    w = pltpu.bitcast((u << sh) & jnp.int32(-65536), f32)
                    b[(0, dt)] = w[:HK]; b[(1, dt)] = w[HK:]
                b11, b12, b21, b22 = b[(0, 0)], b[(0, 1)], b[(1, 0)], b[(1, 1)]
                for i, qv in enumerate((b11 + b22, b11, b12 - b22, b21 - b11, b22, b11 + b12, b21 + b22)):
                    wkv_s[i, a] = qv.astype(bf)
        extract_kv(0)
        HS = S // 2
        @pl.loop(0, HS // 128)
        def _(gi):
            r0 = pl.multiple_of(gi * 128, 128)
            top = pl.ds(r0, 128); bot = pl.ds(HS + r0, 128)
            for t in range(4):
                a11 = c_s[t, top, :].astype(f32); a12 = c_s[4 + t, top, :].astype(f32)
                a21 = c_s[t, bot, :].astype(f32); a22 = c_s[4 + t, bot, :].astype(f32)
                for i, pv_ in enumerate((a11 + a22, a21 + a22, a11 + a12, a21 - a11, a12 - a22)):
                    pc[i, t, top, :] = pv_.astype(bf)

        row = lax.broadcasted_iota(jnp.int32, (sub, sub), 0)
        col = lax.broadcasted_iota(jnp.int32, (sub, sub), 1)
        tri = col <= row

        def hbody(h, _):
            st = {}
            def qload(r0, r1):
                return jnp.concatenate([q_all[2 * h, r0:r1, :], q_all[2 * h + 1, r0:r1, :]], axis=1)
            def kload(r0, r1):
                return jnp.concatenate([k_s[0, r0:r1, :], k_s[1, r0:r1, :]], axis=1)
            def vload(r0, r1):
                return jnp.concatenate([v_s[0, r0:r1, :], v_s[1, r0:r1, :]], axis=1)
            def sp(i, ch):
                rows = slice(ch * sbm, (ch + 1) * sbm)
                if i == 3:
                    lhs = [c_s[t, rows, :] for t in range(4)]
                elif i == 4:
                    lhs = [c_s[4 + t, HS + ch * sbm:HS + (ch + 1) * sbm, :] for t in range(4)]
                else:
                    pi = {1: 0, 2: 1, 5: 2, 6: 3, 7: 4}[i]
                    lhs = [pc[pi, t, rows, :] for t in range(4)]
                w = jnp.concatenate([wkv_s[i - 1, 0], wkv_s[i - 1, 1]], axis=1)
                m = jnp.dot(jnp.concatenate(lhs, axis=1), w, preferred_element_type=f32)
                for blk, sign in {1: ((11, 1), (22, 1)), 2: ((21, 1), (22, -1)), 3: ((12, 1), (22, 1)), 4: ((11, 1), (21, 1)),
                                  5: ((11, -1), (12, 1)), 6: ((22, 1),), 7: ((11, 1),)}[i]:
                    key = ("c", blk, ch)
                    if key not in st:
                        st[key] = [m if sign > 0 else -m, 1]
                    else:
                        st[key][0] = st[key][0] + m if sign > 0 else st[key][0] - m
                        st[key][1] += 1
                    if st[key][1] == {11: 4, 12: 2, 21: 2, 22: 4}[blk]:
                        r = st.pop(key)[0].astype(bf)
                        base = (blk // 10 - 1) * HS + ch * sbm
                        dt = blk % 10 - 1
                        k_s[dt, base:base + sbm, :] = r[:, :128]
                        v_s[dt, base:base + sbm, :] = r[:, 128:]
            def qk(i, j):
                if j < i:
                    s = lax.dot_general(qload(i*bq, (i+1)*bq), kload(j*bq, (j+1)*bq), NT, preferred_element_type=f32)
                    st[("s", i, j)] = s
                    mj = jnp.max(s, axis=1, keepdims=True)
                else:
                    parts = [[] for _ in range(nsub)]
                    for t in range(nsub):
                        r0 = t * sub
                        s = lax.dot_general(qload(i*bq + r0, (i+1)*bq), kload(j*bq + r0, j*bq + r0 + sub), NT, preferred_element_type=f32)
                        parts[t].append(jnp.where(tri, s[:sub], NEG))
                        for r in range(t + 1, nsub):
                            parts[r].append(s[(r-t)*sub:(r-t+1)*sub])
                    st[("sd", i)] = parts
                    ms = [jnp.max(functools.reduce(jnp.maximum, parts[r]), axis=1, keepdims=True) for r in range(nsub)]
                    mj = jnp.concatenate(ms, axis=0)
                st[("m", i)] = mj if ("m", i) not in st else jnp.maximum(st[("m", i)], mj)
            def pv(i, j):
                m = st[("m", i)]
                if j < i:
                    sfull = st.pop(("s", i, j))
                    for c0 in range(0, bq, pv_split):
                        p = jnp.exp2(sfull[:, c0:c0 + pv_split] - m)
                        lj = functools.reduce(jnp.add, [p[:, t*sub:(t+1)*sub] for t in range(pv_split // sub)])
                        o = jnp.dot(p.astype(bf), vload(j*bq + c0, j*bq + c0 + pv_split), preferred_element_type=f32)
                        st[("l", i)] = lj if ("l", i) not in st else st[("l", i)] + lj
                        st[("o", i)] = o if ("o", i) not in st else st[("o", i)] + o
                else:
                    parts = st.pop(("sd", i))
                    for r in range(nsub):
                        rows = slice(r*sub, (r+1)*sub)
                        w = (r+1)*sub
                        ps = [jnp.exp2(x - m[rows]) for x in parts[r]]
                        lj = functools.reduce(jnp.add, ps)
                        p = jnp.concatenate(ps, axis=1) if r > 0 else ps[0]
                        o = jnp.dot(p.astype(bf), vload(j*bq, j*bq + w), preferred_element_type=f32)
                        if ("l", i) in st:
                            lj = lj + st[("l", i)][rows]; o = o + st[("o", i)][rows]
                        l = jnp.sum(lj, axis=1, keepdims=True)
                        rl = pl.reciprocal(l, approx=True)
                        rl = rl * (2.0 - l * rl)
                        ctx = (o * rl).astype(bf)
                        rr = slice(i*bq + r*sub, i*bq + (r+1)*sub)
                        q_all[2 * h, rr, :] = ctx[:, :128]
                        q_all[2 * h + 1, rr, :] = ctx[:, 128:]
            att = []
            for i in range(nq - 2, -2, -1):
                a = [("qk", i, j) for j in range(i+1)] if i >= 0 else []
                b = [("pv", i+1, j) for j in range(i+2)]
                for t in range(max(len(a), len(b))):
                    if t < len(a): att.append(a[t])
                    if t < len(b): att.append(b[t])
            P = sorder
            seq = ([("sp", i, 0) for i in P] + [("qk", 3, 0), ("qk", 3, 2)] + [("sp", i, 1) for i in P]
                   + [("qk", 3, 1), ("qk", 3, 3), ("ex",)] + att)
            for op in seq:
                if op[0] == "sp": sp(*op[1:])
                elif op[0] == "qk": qk(*op[1:])
                elif op[0] == "pv": pv(*op[1:])
                elif op[0] == "ex": extract_kv(jnp.minimum(h + 1, H - 1))
        lax.fori_loop(0, H, hbody, None)

        start('oproj')
        dmas["wo"].wait(); dmas["g"].wait()
        nt_per = oproj_bm // 128
        def obody(m, _):
            for u in range(nt_per):
                r0 = pl.multiple_of(m * oproj_bm + u * 128, 128)
                rows = pl.ds(r0, 128)
                ye = jnp.concatenate([ys[0, rows, :], ys[2, rows, :]], axis=1)
                yo = jnp.concatenate([ys[1, rows, :], ys[3, rows, :]], axis=1)
                ev = lax.dot_general(g[0], ye, NT, preferred_element_type=f32)
                od = lax.dot_general(g[1], yo, NT, preferred_element_type=f32)
                at = jnp.concatenate([ev + od, ev - od], axis=0)
                ctx = jnp.concatenate([q_all[t, rows, :] for t in range(32)], axis=1)
                w = jnp.concatenate([woT[hh] for hh in range(H)], axis=1)
                bt = lax.dot_general(w, ctx, NT, preferred_element_type=f32)
                tt = jnp.concatenate([at, bt], axis=0)
                for c in range(7):
                    out_s[rows, c * 128:(c + 1) * 128] = tt[c * 128:(c + 1) * 128].T.astype(bf)
                pltpu.make_async_copy(out_s.at[rows], out_hbm.at[rows], osem.at[m * nt_per + u]).start()
        lax.fori_loop(0, S // oproj_bm, obody, None)
        def owait(m, _):
            rows = pl.ds(pl.multiple_of(m * 128, 128), 128)
            pltpu.make_async_copy(out_s.at[rows], out_hbm.at[rows], osem.at[m]).wait()
        lax.fori_loop(0, S // 128, owait, None)

    def fn(A_x, A_w_r, A_w_i, B_x, B_c_kv, B_w_q, B_w_uk, B_w_uv, B_w_o):
        V = pltpu.VMEM
        scratch = ([V((M, S), bf), V((DF, S), bf), V((DF, S), bf), V((480, HM), bf), V((16, 128, 256), bf), V((16, 128, 256), bf),
                    V((2, HM, 256), bf), V((128, 128), bf), V((480, S), f32), V((2, 16, 128, 256), bf), V((2, 2, 16, 128, 128), f32),
                    V((2, 16, 256, 128), f32), V((4, S, 128), bf)]
            + [V((7, S // 2, 128), bf), V((7, S // 2, HM - 128), bf)] + [V((8, S, 128), bf), V((2, M*H, 128), bf), V((2, DC*H, 128), bf), V((2, DC*H, 128), bf)]
            + [V((7, 2, HM, 128), bf), V((7, 2, DC // 2, 128), bf), V((32, S, 128), bf), V((2, S, 128), bf), V((2, S, 128), bf), V((S, 896), bf),
               V((M, S), bf), V((H, M, D), bf), V((5, 4, S // 2, 128), bf),
               pltpu.SemaphoreType.DMA((48,)), pltpu.SemaphoreType.DMA((16,))])
        out = pl.pallas_call(kern, in_specs=[pl.BlockSpec(memory_space=pl.ANY)]*14, out_specs=pl.BlockSpec(memory_space=pl.ANY),
            out_shape=jax.ShapeDtypeStruct((S, 896), bf), scratch_shapes=scratch,
            compiler_params=pltpu.CompilerParams(vmem_limit_bytes=120<<20, flags=flags))(
            A_x.reshape(S, M).T, A_w_r.T, A_w_i.T, B_x.reshape(S, M).T, B_c_kv.reshape(S, DC), B_w_q.reshape(M*H, D),
            B_w_uk.reshape(DC*H, D), B_w_uv.reshape(DC*H, D), B_w_o.transpose(0, 2, 1), *consts)
        return out.reshape(1, S, 896)
    return fn


@jax.jit
def pallas_concat_heads__spectral_gfnet__compressed_kv_cla__prompt_kernel(
    A_x, A_w_r, A_w_i, B_x, B_c_kv, B_w_q, B_w_uk, B_w_uv, B_w_o,
):
    return make()(A_x, A_w_r, A_w_i, B_x, B_c_kv, B_w_q, B_w_uk, B_w_uv, B_w_o)
```
